```python
import os as _os
_os.environ.setdefault("JAX_PLATFORMS", "cpu")
import jax
import jax.numpy as jnp

def _softmax(x, axis=-1):
    return jax.nn.softmax(x, axis=axis)
def _gelu(x):
    return jax.nn.gelu(x, approximate=True)
def _silu(x):
    return jax.nn.silu(x)
def _sigmoid(x):
    return jax.nn.sigmoid(x)
def _layernorm(x, axis=-1, eps=1e-5):
    m = jnp.mean(x, axis=axis, keepdims=True)
    v = jnp.var(x, axis=axis, keepdims=True)
    return (x - m) / jnp.sqrt(v + eps)
def _scatter_add(tgt, idx, src, axis=0):
    return tgt.at[idx].add(src)
def _segment_sum(src, seg, n):
    return jax.ops.segment_sum(src, seg, n)
class _Rng:
    def __init__(self, key):
        self._k = key
    def _next(self):
        self._k, sub = jax.random.split(self._k)
        return sub
    def normal(self, shape):
        return jax.random.normal(self._next(), shape, dtype=jnp.bfloat16)
    def randint(self, lo, hi, shape):
        return jax.random.randint(self._next(), shape, lo, hi, dtype=jnp.int32)
    def uniform(self, shape, lo=0.0, hi=1.0):
        return jax.random.uniform(self._next(), shape, jnp.bfloat16, lo, hi)
    def permutation(self, n):
        return jax.random.permutation(self._next(), n)


kernel_name = 'interleave_layers__spectral_gfnet__dense_activation_gelu__prompt'

def setup_inputs():
    _rng = _Rng(jax.random.key(int.from_bytes(__import__("os").urandom(4), "little")))
    _w = (lambda a: (lambda t: t.astype(jnp.bfloat16) if jnp.issubdtype(t.dtype, jnp.floating) else t)(jnp.asarray(a)))
    def _A_setup():
        B, S, D = 1, 2048, 640
        Df = D // 2 + 1
        return {
            "x": _w((lambda *s: _rng.normal(s) * 0.05)(B, S, D)),
            "w_r": _w((lambda *s: _rng.normal(s) * 0.2)(S, Df) * 0.02),
            "w_i": _w((lambda *s: _rng.normal(s) * 0.2)(S, Df) * 0.02),
        }
    _A_in = _A_setup()

    def _B_setup():
        B, S, D, F = 1, 2048, 640, 1728
        return {
            "x": _w((lambda *s: _rng.normal(s) * 0.05)(B, S, D)),
            "w1": _w((lambda *s: _rng.normal(s) * 0.1)(D, F) * (D ** -0.5)),
            "b1": _w((lambda *s: _rng.normal(s) * 0.1)(F) * 0.01),
            "w2": _w((lambda *s: _rng.normal(s) * 0.1)(F, D) * (F ** -0.5)),
            "b2": _w((lambda *s: _rng.normal(s) * 0.1)(D) * 0.01),
        }
    _B_in = _B_setup()

    return {
        "A_x": _A_in["x"],
        "A_w_r": _A_in["w_r"],
        "A_w_i": _A_in["w_i"],
        "B_x": _B_in["x"],
        "B_w1": _B_in["w1"],
        "B_b1": _B_in["b1"],
        "B_w2": _B_in["w2"],
        "B_b2": _B_in["b2"],
    }

def reference(A_x, A_w_r, A_w_i, B_x, B_w1, B_b1, B_w2, B_b2):
    def _A_ref(x, w_r, w_i):
        B, S, D = x.shape
        X = (lambda x, axes=(-2,-1): jnp.fft.rfft2(x.astype(jnp.float32), axes=axes))(x, axes=(-2, -1))
        W = w_r + 1j * w_i
        X = X * W
        y = (lambda x, s, axes=(-2,-1): jnp.fft.irfft2(x, s=s, axes=axes).astype(jnp.bfloat16))(X, (S, D), axes=(-2, -1))
        return y

    def _B_ref(x, w1, b1, w2, b2):
        h = jnp.einsum("bsd,df->bsf", x, w1) + b1
        h = _gelu(h)
        return jnp.einsum("bsf,fd->bsd", h, w2) + b2

    x = A_x
    x = x + _A_ref(_layernorm(x, axis=-1), A_w_r, A_w_i)
    x = x + _B_ref(_layernorm(x, axis=-1), B_w1, B_b1, B_w2, B_b2)
    x = x + _A_ref(_layernorm(x, axis=-1), A_w_r, A_w_i)
    x = x + _B_ref(_layernorm(x, axis=-1), B_w1, B_b1, B_w2, B_b2)
    return x
```

```python
import math
import os
import numpy as np
import jax
import jax.numpy as jnp
from jax import lax
import jax.experimental.pallas as pl
import jax.experimental.pallas.tpu as pltpu

S, D, F, DF = 2048, 640, 1728, 321
NA, NB = 32, 64
BF = jnp.bfloat16
F32 = jnp.float32
U32 = jnp.uint32

C1, C2 = math.cos(2 * math.pi / 5), math.cos(4 * math.pi / 5)
S1, S2 = math.sin(2 * math.pi / 5), math.sin(4 * math.pi / 5)
K5 = math.sqrt(5.0) / 4.0
R21 = S2 / S1
AORD = [4 * a2 + a1 for a1 in range(4) for a2 in range(8)]
APOS = {a: p for p, a in enumerate(AORD)}


def _fwd5(z):
    z0, z1, z2, z3, z4 = z
    s14 = z1 + z4; d14 = z1 - z4; s23 = z2 + z3; d23 = z2 - z3
    u = s14 + s23
    t0 = z0 + u
    m = z0 - 0.25 * u
    n = K5 * (s14 - s23)
    return t0, m + n, d14 + R21 * d23, m - n, R21 * d14 - d23


def _inv5(q):
    q0, q1r, q1i, q2r, q2i = q
    u = q1r + q2r
    y0 = q0 + u
    m = q0 - 0.25 * u
    n = K5 * (q1r - q2r)
    a1 = m + n; a2 = m - n
    b1 = q1i + R21 * q2i
    b2 = R21 * q1i - q2i
    return y0, a1 - b1, a2 - b2, a2 + b2, a1 + b1


_GROUPS = {1: [(1, 6), (9, 4)], 2: [(7, 2), (3, 8)], 0: [(5, 10)]}


def _lane_plan():
    out = {}
    for cl, prs in _GROUPS.items():
        kd = []
        for (rh, rl) in prs:
            for m in range(32):
                kd += [rh + 10 * m, rl + 10 * m]
        out[cl] = np.array(kd, np.int64)
    return out[0], out[1], out[2]


def _build_consts():
    kd0, kd1, kd2 = _lane_plan()
    n = np.arange(D)
    eye = np.eye(D)

    def cs(kd):
        th = 2 * np.pi * np.outer(n, kd) / D
        return np.cos(th), np.sin(th)
    c0, s0 = cs(kd0); c1, s1 = cs(kd1); c2, s2 = cs(kd2)
    s0[:, kd0 == 320] = 0.0
    tiles = [eye[:, 128 * a:128 * (a + 1)] for a in range(5)]
    Ffull = np.concatenate([c0, -s0, c1, -s1, c2, -s2], axis=1)
    Fm = np.linalg.solve(np.concatenate(_fwd5(tiles), axis=1), Ffull)
    kap = lambda kd: np.where(kd == 320, 1.0, 2.0)
    Gfull = np.concatenate([(c0 * kap(kd0)).T, (-s0 * kap(kd0)).T, (c1 * kap(kd1)).T, (-s1 * kap(kd1)).T,
                            (c2 * kap(kd2)).T, (-s2 * kap(kd2)).T], axis=0) / (D * S)
    Gm = np.linalg.solve(np.concatenate(_inv5(tiles), axis=1).T, Gfull.T).T
    Mf = np.zeros((NA, 128, 128)); Mi = np.zeros((NA, 128, 128))
    b = np.arange(64)
    kr = 16 * (b // 8) + 2 * (b % 8); ki = kr + 1
    for c in range(NA):
        pos = np.arange(64)
        e = pos if c % 2 == 0 else 8 * (pos // 8) + (pos % 8 + 4) % 8
        th = 2 * np.pi * np.outer(c + 32 * e, b) / S
        co, si = np.cos(th), np.sin(th)
        Mf[c][np.ix_(pos, kr)] = co; Mf[c][np.ix_(pos, ki)] = si
        Mf[c][np.ix_(64 + pos, kr)] = -si; Mf[c][np.ix_(64 + pos, ki)] = co
        Mi[c][np.ix_(b, pos)] = co.T; Mi[c][np.ix_(b, 64 + pos)] = -si.T
        Mi[c][np.ix_(64 + b, pos)] = si.T; Mi[c][np.ix_(64 + b, 64 + pos)] = co.T
    L = np.zeros((2, 128, 128))
    for par in range(2):
        for m in range(128):
            gam, j = m // 8, m % 8
            c = 2 * gam + ((j >= 4) if par == 0 else (j < 4))
            L[par, m, c + 32 * (j % 4)] = 1.0
    bf = lambda x: np.asarray(x, dtype=np.float32).astype(BF)
    def pack3(M):
        out = np.zeros((256, 640))
        out[0:128, 0:128] = M[0:128, 0:128]
        out[:, 128:384] = M[128:384, 128:384]
        out[:, 384:640] = M[384:640, 384:640]
        return bf(out)
    def w32(a):
        u = np.asarray(a).view(np.uint16).astype(np.uint32)
        return np.ascontiguousarray(u[..., 0::2, :] | (u[..., 1::2, :] << 16))
    return dict(Fc=w32(pack3(Fm)), Gc=w32(pack3(Gm)), Mf=w32(bf(Mf)), Mi=w32(bf(Mi)), L=w32(bf(L)))


class _Cplx:
    @staticmethod
    def add(a, b): return (a[0] + b[0], a[1] + b[1])
    @staticmethod
    def sub(a, b): return (a[0] - b[0], a[1] - b[1])
    @staticmethod
    def addsubi(a, b):
        return (a[0] - b[1], a[1] + b[0]), (a[0] + b[1], a[1] - b[0])
    @staticmethod
    def muli(a, sg):
        return (-a[1], a[0]) if sg > 0 else (a[1], -a[0])
    @staticmethod
    def mul(a, c, s):
        if abs(abs(c) - abs(s)) < 1e-12:
            if s * c > 0:
                return (c * (a[0] - a[1]), c * (a[0] + a[1]))
            return (c * (a[0] + a[1]), c * (a[1] - a[0]))
        return (c * a[0] - s * a[1], c * a[1] + s * a[0])


class _Half:
    def __init__(self, sig):
        self.sig = sig
    def J(self, v): return pltpu.roll(v, 64, 1) * self.sig
    def add(self, a, b): return a + b
    def sub(self, a, b): return a - b
    def addsubi(self, a, b):
        jb = self.J(b)
        return a + jb, a - jb
    def mul(self, a, c, s): return c * a + s * self.J(a)
    def muli(self, a, sg): return self.J(a) if sg > 0 else -self.J(a)


def _fft(x, A, sign):
    N = len(x)
    if N == 1:
        return [x[0]]
    if N == 2:
        return [A.add(x[0], x[1]), A.sub(x[0], x[1])]
    E = _fft(x[0::2], A, sign); O1 = _fft(x[1::4], A, sign); O3 = _fft(x[3::4], A, sign)
    X = [None] * N
    for k in range(N // 4):
        t1, t3 = O1[k], O3[k]
        if k:
            a1 = sign * 2 * math.pi * k / N; a3 = 3 * a1
            t1 = A.mul(t1, math.cos(a1), math.sin(a1)); t3 = A.mul(t3, math.cos(a3), math.sin(a3))
        s = A.add(t1, t3); d = A.sub(t1, t3)
        X[k] = A.add(E[k], s); X[k + N // 2] = A.sub(E[k], s)
        p, m = A.addsubi(E[k + N // 4], d)
        if sign > 0:
            X[k + N // 4], X[k + 3 * N // 4] = p, m
        else:
            X[k + N // 4], X[k + 3 * N // 4] = m, p
    return X


def _tw(A, v, a1, c2, sign):
    n = (a1 * c2) % 32
    if n == 0:
        return v
    if n == 8:
        return A.muli(v, sign)
    ang = sign * 2 * math.pi * n / 32
    return A.mul(v, math.cos(ang), math.sin(ang))


def _dot(a, b):
    return jnp.dot(a, b, preferred_element_type=F32)


def _dot_nt(a, b):
    return lax.dot_general(a, b, (((1,), (1,)), ((), ())), preferred_element_type=F32)


def _ln(x):
    m = jnp.sum(x, axis=1, keepdims=True) * (1.0 / D)
    d = x - m
    v = jnp.sum(d * d, axis=1, keepdims=True) * (1.0 / D)
    return d * lax.rsqrt(v + 1e-5)


def _gelu(h):
    inner = h * (0.7978845608028654 + (0.7978845608028654 * 0.044715) * (h * h))
    hh = 0.5 * h
    return hh + hh * jnp.tanh(inner)


def _run(gen):
    for _ in gen:
        pass


def _count(make):
    n = 0
    for _ in make():
        n += 1
    return n


def _pk(v):
    return pltpu.bitcast(v, U32)


def _upk(w):
    return pltpu.bitcast(w, BF)


def _kernel(x_hbm, wr_hbm, wi_hbm, w1_hbm, b1_ref, w2_hbm, b2_ref,
            Fc_hbm, Gc_hbm, Mf_hbm, Mi_hbm, L_hbm,
            o_hbm,
            XI, O, Wraw, w1_ref, w2_ref, Fc, Gc, Mf_ref, Mi_ref, L_ref, b1f, b2f,
            X, V, H12, H0, Wr12, Wi12, Wa0, Wb0, Wst, XN, G, Ys, Zs,
            sx, sw, sm, so):
    lane = lax.broadcasted_iota(jnp.int32, (8, 128), 1)
    sub = lax.broadcasted_iota(jnp.int32, (8, 128), 0)
    lo8 = lane < 64
    sig8 = jnp.where(lo8, -1.0, 1.0).astype(F32)

    cx = [pltpu.make_async_copy(x_hbm.at[:, g], XI.at[g], sx.at[g]) for g in range(8)]
    cw = [pltpu.make_async_copy((wr_hbm, wi_hbm)[k].at[:, pl.ds(512 * q, 512)], Wraw.at[k, q], sw.at[2 * q + k])
          for q in range(4) for k in range(2)]
    cF = pltpu.make_async_copy(Fc_hbm, Fc, sm.at[0])
    cG = pltpu.make_async_copy(Gc_hbm, Gc, sm.at[1])
    cL = pltpu.make_async_copy(L_hbm, L_ref, sm.at[2])
    cMf = [pltpu.make_async_copy(Mf_hbm.at[pl.ds(8 * q, 8)], Mf_ref.at[pl.ds(8 * q, 8)], sm.at[3 + q]) for q in range(4)]
    cMi = [pltpu.make_async_copy(Mi_hbm.at[pl.ds(8 * q, 8)], Mi_ref.at[pl.ds(8 * q, 8)], sm.at[7 + q]) for q in range(4)]
    cw1 = [pltpu.make_async_copy(w1_hbm.at[pl.ds(a, n)], w1_ref.at[pl.ds(a, n)], sm.at[11 + i])
           for i, (a, n) in enumerate(((0, 640), (640, 512), (1152, 576)))]
    cw2 = [pltpu.make_async_copy(w2_hbm.at[:, pl.ds(128 * n, 128)], w2_ref.at[:, pl.ds(128 * n, 128)], sm.at[14 + n])
           for n in range(5)]
    cx[0].start(); cF.start(); cx[1].start()

    b1f[...] = jnp.broadcast_to(b1_ref[...].astype(F32)[None, :], (8, F))
    b2f[...] = jnp.broadcast_to(b2_ref[...].astype(F32)[None, :], (8, D))
    F0_ref = lambda: _upk(Fc[0:64, 0:128])
    F1_ref = lambda: _upk(Fc[0:128, 128:384])
    F2_ref = lambda: _upk(Fc[0:128, 384:640])
    G0_ref = lambda: _upk(Gc[0:64, 0:128])
    G1_ref = lambda: _upk(Gc[0:128, 128:384])
    G2_ref = lambda: _upk(Gc[0:128, 384:640])

    def wprep(q):
        lo4 = sub < 4
        for tp in range(2):
            outs = []
            for par in range(2):
                tl = 2 * tp + par
                Lm = _upk(L_ref[par])
                o = []
                for k in range(2):
                    Wst[k, par, 0:160, :] = _pk(Wraw[k, q, 0:320, 128 * tl:128 * tl + 128])
                    Wst[k, par, 160:161, :] = pltpu.bitcast(
                        Wraw[k, q, 320:321, 128 * tl:128 * tl + 128].astype(F32), U32) >> 16

                    def tile(cl):
                        ws = []
                        for (rh, rl) in _GROUPS[cl]:
                            hi = Wst[k, par, pl.ds(rh // 2, 32, stride=5), :]
                            lo = Wst[k, par, pl.ds(rl // 2, 32, stride=5), :]
                            ws.append((hi >> 16) | (lo << 16))
                        return jnp.concatenate(ws, axis=0) if len(ws) > 1 else ws[0]
                    t1 = _dot_nt(Lm, _upk(tile(1)))
                    t2 = _dot_nt(Lm, _upk(tile(2)))
                    w0 = tile(0)
                    w0 = jnp.concatenate([w0, w0] if k == 0 else [w0 ^ jnp.uint32(0x80008000), w0], axis=0)
                    t0 = _dot_nt(Lm, _upk(w0))
                    o += [t1, t2, t0]
                outs.append(o)
                yield
            G8 = 8 * (2 * q + tp)
            dst = [(Wr12, 0), (Wr12, 128), (Wa0, 0), (Wi12, 0), (Wi12, 128), (Wb0, 0)]
            for ti in range(6):
                ref, l0 = dst[ti]
                for gam in range(16):
                    A_ = outs[0][ti][8 * gam:8 * gam + 8]; B_ = outs[1][ti][8 * gam:8 * gam + 8]
                    ref[2 * gam, G8:G8 + 8, l0:l0 + 128] = jnp.where(lo4, A_, B_)
                    ref[2 * gam + 1, G8:G8 + 8, l0:l0 + 128] = jnp.where(lo4, B_, A_)
            yield

    sigp = -sig8

    def jp(v):
        return pltpu.roll(v, 64, 1) * sigp

    def rowsum(x):
        return jnp.sum(x, axis=1, keepdims=True)

    def xin(g, a1):
        return jnp.concatenate([XI[g, AORD[8 * a1 + a2]].astype(F32) for a2 in range(8)], axis=0)

    S1SQ = S1 * S1

    def stC1(g, slot, first=False):
        for a1 in range(4):
            r0 = 64 * a1
            x = xin(g, a1) if first else X[g, r0:r0 + 64, :]
            t0, t1r, t1i, t2r, t2i = _fwd5([x[:, 128 * a:128 * (a + 1)] for a in range(5)])
            U1 = _dot(jnp.concatenate([t1r, t1i], axis=1).astype(BF), F1_ref())
            U2 = _dot(jnp.concatenate([t2r, t2i], axis=1).astype(BF), F2_ref())
            p = (t1r * t1r + t2r * t2r) + S1SQ * (t1i * t1i + t2i * t2i)
            m5 = rowsum(t0) * (1.0 / 128)
            yield
            t0c = t0 - m5
            U0 = _dot(t0c.astype(BF), F0_ref())
            v = rowsum(2.0 * p + t0c * t0c)
            yield
            rs = jnp.exp2(-0.5 * jnp.log2(v * (1.0 / (5 * D)) + 1e-5))
            U0 = U0 * rs; U1 = U1 * rs; U2 = U2 * rs
            x0 = [(U0[8 * a2:8 * a2 + 8], jp(U0[8 * a2:8 * a2 + 8])) for a2 in range(8)]
            for cl, Uc in ((1, U1), (2, U2)):
                xs = [(Uc[8 * a2:8 * a2 + 8, :128], Uc[8 * a2:8 * a2 + 8, 128:]) for a2 in range(8)]
                Y = _fft(xs, _Cplx, -1)
                for c2 in range(8):
                    w = _tw(_Cplx, Y[c2], a1, c2, -1)
                    Ys[slot, 2 * cl - 1, a1, c2] = w[0]; Ys[slot, 2 * cl, a1, c2] = w[1]
                yield
            Y = _fft(x0, _Cplx, -1)
            for c2 in range(8):
                Ys[slot, 0, a1, c2] = _tw(_Cplx, Y[c2], a1, c2, -1)[0]
            yield

    def stC2(g, slot):
        r0 = pl.multiple_of(8 * g, 8)
        for c2 in range(8):
            y0 = [Ys[slot, 0, a1, c2] for a1 in range(4)]
            x0 = [(y, jp(y)) for y in y0]
            for cl in (1, 2, 0):
                if cl:
                    xs = [(Ys[slot, 2 * cl - 1, a1, c2], Ys[slot, 2 * cl, a1, c2]) for a1 in range(4)]
                else:
                    xs = x0
                Xo = _fft(xs, _Cplx, -1)
                for c1 in range(4):
                    V[c2 + 8 * c1, cl, pl.ds(r0, 8), :] = pltpu.pack_elementwise([Xo[c1][0], Xo[c1][1]], packed_dtype=BF)
            yield

    def stA1(g, slot):
        r0 = pl.multiple_of(8 * g, 8)
        for c2 in range(8):
            h0 = [H0[c2 + 8 * c1, pl.ds(r0, 8), :] for c1 in range(4)]
            x0 = [(h, jp(h)) for h in h0]
            for cl in (1, 2):
                l0 = 128 * (cl - 1)
                Z = _fft([(H12[c2 + 8 * c1, pl.ds(r0, 8), l0:l0 + 128], H12[c2 + 8 * c1, pl.ds(64 + r0, 8), l0:l0 + 128])
                          for c1 in range(4)], _Cplx, +1)
                for a1 in range(4):
                    v = _tw(_Cplx, Z[a1], a1, c2, +1)
                    Zs[slot, 2 * cl - 1, a1, c2] = v[0]; Zs[slot, 2 * cl, a1, c2] = v[1]
            Z = _fft(x0, _Cplx, +1)
            for a1 in range(4):
                Zs[slot, 0, a1, c2] = _tw(_Cplx, Z[a1], a1, c2, +1)[0]
            yield

    def stA2(g, slot, xslot, first=False):
        for a1 in range(4):
            r0 = 64 * a1
            z0 = [Zs[slot, 0, a1, c2] for c2 in range(8)]
            x0 = [(z, jp(z)) for z in z0]
            tl = [None] * 5
            for cl in (1, 2):
                Vo = _fft([(Zs[slot, 2 * cl - 1, a1, c2], Zs[slot, 2 * cl, a1, c2]) for c2 in range(8)], _Cplx, +1)
                for ri in range(2):
                    tl[2 * cl - 1 + ri] = jnp.concatenate([o[ri] for o in Vo], axis=0)
            Vo = _fft(x0, _Cplx, +1)
            tl[0] = jnp.concatenate([o[0] for o in Vo], axis=0)
            q1 = _dot(jnp.concatenate([tl[1], tl[2]], axis=1).astype(BF), G1_ref())
            q2 = _dot(jnp.concatenate([tl[3], tl[4]], axis=1).astype(BF), G2_ref())
            q0 = _dot(tl[0].astype(BF), G0_ref())
            yield
            ys = _inv5([q0, q1[:, :128], q1[:, 128:], q2[:, :128], q2[:, 128:]])
            x1 = (xin(g, a1) if first else X[g, r0:r0 + 64, :]) + jnp.concatenate(ys, axis=1)
            X[g, r0:r0 + 64, :] = x1
            m = rowsum(x1) * (1.0 / D)
            yield
            d = X[g, r0:r0 + 64, :] - m
            v = rowsum(d * d)
            yield
            rs = jnp.exp2(-0.5 * jnp.log2(v * (1.0 / D) + 1e-5))
            XN[xslot, r0:r0 + 64, :] = ((X[g, r0:r0 + 64, :] - m) * rs).astype(BF)
            yield

    def stB1(g, slot):
        for j in range(14):
            n0, n1 = 128 * j, min(128 * j + 128, F)
            h = _dot_nt(XN[slot], w1_ref[n0:n1, :]) + b1f[0:1, n0:n1]
            G[:, n0:n1] = _gelu(h).astype(BF)
            yield

    def stB2(g, slot, last=False):
        for n in range(5):
            for rh in range(2):
                r0 = 128 * rh
                o = _dot(G[r0:r0 + 128, :], w2_ref[:, 128 * n:128 * n + 128]) + b2f[0:1, 128 * n:128 * n + 128]
                x2 = X[g, r0:r0 + 128, 128 * n:128 * n + 128] + o
                if last:
                    for pp in range(16):
                        O[g, AORD[16 * rh + pp], :, 128 * n:128 * n + 128] = x2[8 * pp:8 * pp + 8].astype(BF)
                else:
                    X[g, r0:r0 + 128, 128 * n:128 * n + 128] = x2
                yield

    def interleave(main, fillers):
        live = [[f, q, 0.0] for f, q in fillers]
        for _ in main:
            nxt = []
            for e in live:
                e[2] += e[1]
                alive = True
                while e[2] >= 1.0 - 1e-9:
                    e[2] -= 1.0
                    try:
                        next(e[0])
                    except StopIteration:
                        alive = False
                        break
                if alive:
                    nxt.append(e)
            live = nxt
        for e in live:
            _run(e[0])

    sig64 = jnp.where(lax.broadcasted_iota(jnp.int32, (64, 128), 1) < 64, 1.0, -1.0).astype(F32)

    def s_phase(first):
        GP = 2
        NG = NA // GP
        Zq = {}; Y = {}; Hh = {}
        cs = lambda p: [GP * p + u for u in range(GP)] if 0 <= p < NG else []
        for i in range(NG + 3):
            if first and i < NG and i % 4 == 0:
                cMf[i // 4].wait(); cMi[i // 4].wait()
                if i == 0:
                    cw1[2].start(priority=1)
                if i == 4:
                    for c_ in cw2:
                        c_.start(priority=1)
            for c in cs(i - 3):
                h12, h0 = Hh.pop(c)
                H12[c] = h12; H0[c] = h0
            a = {}; b = {}
            for c in cs(i - 2):
                a[c] = _dot(_upk(Mi_ref[c]), Y[c][0])
            for c in cs(i):
                v12 = jnp.concatenate([_upk(V[c, 1]), _upk(V[c, 2])], axis=1)
                b[c] = _dot(_upk(Mf_ref[c]), v12)
            for c in cs(i - 2):
                Hh[c] = (a[c], _dot(_upk(Mi_ref[c, 0:32]), Y.pop(c)[1]))
            for c in cs(i):
                Zq[c] = (b[c], _dot(_upk(Mf_ref[c, 0:32]), _upk(V[c, 0])))
            for c in cs(i - 1):
                z12, z0 = Zq.pop(c)
                Zr, Zi = z12[0:64], z12[64:128]
                wr = Wr12[c]; wi = Wi12[c]
                y12 = jnp.concatenate([Zr * wr - Zi * wi, Zr * wi + Zi * wr], axis=0).astype(BF)
                y0 = z0 * Wa0[c] + pltpu.roll(z0, 64, 1) * Wb0[c]
                st = jnp.concatenate([y0, pltpu.roll(y0, 64, 1) * sig64], axis=0).astype(BF)
                Y[c] = (y12, st)

    with jax.named_scope('ph1'):
        P1 = dict(priority=1)
        cx[0].wait()
        for g in range(2, 8):
            cx[g].start()
        cL.start()
        for c in cw:
            c.start(**P1)
        cF.wait(); cx[1].wait()
        interleave(stC1(0, 0, True), [(stC1(1, 1, True), 1.0)])
        for g in (2, 4, 6):
            cx[g].wait(); cx[g + 1].wait()
            if g == 4:
                for q in range(2):
                    cMf[q].start(**P1); cMi[q].start(**P1)
            if g == 6:
                for q in range(2, 4):
                    cMf[q].start(**P1); cMi[q].start(**P1)
                cG.start(**P1)
            interleave(stC1(g, g % 4, True), [(stC1(g + 1, (g + 1) % 4, True), 1.0),
                                               (stC2(g - 2, (g - 2) % 4), 0.4), (stC2(g - 1, (g - 1) % 4), 0.4)])
        interleave(stC2(6, 2), [(stC2(7, 3), 1.0)])
    with jax.named_scope('wprep'):
        cL.wait()
        for q in range(4):
            cw[2 * q].wait(); cw[2 * q + 1].wait()
            if q == 1:
                cw1[0].start(**P1)
            if q == 3:
                cw1[1].start(**P1)
            _run(wprep(q))

    with jax.named_scope('s1'):
        s_phase(True)

    QA1 = float(os.environ.get('QA1', 8 / 14)); QC1 = float(os.environ.get('QC1', 20 / 14))
    QA2 = float(os.environ.get('QA2', 16 / 10)); QC2 = float(os.environ.get('QC2', 8 / 10))

    def out_copy(g):
        return pltpu.make_async_copy(O.at[g], o_hbm.at[:, g], so.at[g])

    def mlp_phase(last):
        first = not last
        if first:
            cG.wait()
        _run(stA1(0, 0))
        _run(stA2(0, 0, 0, first))
        def body(g, hasC, hasA, wwait=False):
            f1 = []; f2 = []
            if hasC:
                f1.append((stC1(g - 1, 0), QC1)); f2.append((stC2(g - 1, 0), QC2))
            if hasA:
                f1.append((stA1(g + 1, 0), QA1)); f2.append((stA2(g + 1, 0, (g + 1) % 2, first), QA2))
            if wwait:
                for c in cw1:
                    c.wait()
            interleave(stB1(g, g % 2), f1)
            if wwait:
                for c in cw2:
                    c.wait()
            interleave(stB2(g, g % 2, last), f2)
            if last:
                out_copy(g).start()
        if last:
            lax.fori_loop(0, 7, lambda g, c: (body(g, False, True), c)[1], 0)
            body(7, False, False)
        else:
            body(0, False, True, wwait=True)
            lax.fori_loop(1, 7, lambda g, c: (body(g, True, True), c)[1], 0)
            body(7, True, False)
            _run(stC1(7, 0))
            _run(stC2(7, 0))

    with jax.named_scope('ph2'):
        mlp_phase(False)
    with jax.named_scope('s2'):
        s_phase(False)
    with jax.named_scope('ph3'):
        mlp_phase(True)
    for g in range(8):
        out_copy(g).wait()


_K = None


@jax.jit
def pallas_interleave_layers__spectral_gfnet__dense_activation_gelu__prompt_kernel(A_x, A_w_r, A_w_i, B_x, B_w1, B_b1, B_w2, B_b2):
    global _K
    if _K is None:
        _K = _build_consts()
    K = _K
    consts = [K[n] for n in ('Fc', 'Gc', 'Mf', 'Mi', 'L')]
    any_spec = pl.BlockSpec(memory_space=pl.ANY)
    vmem_spec = pl.BlockSpec(memory_space=pltpu.VMEM)
    out = pl.pallas_call(
        _kernel,
        out_shape=jax.ShapeDtypeStruct((NA, 8, 8, D), BF),
        in_specs=[any_spec, any_spec, any_spec, any_spec, vmem_spec, any_spec, vmem_spec] + [any_spec] * 5,
        out_specs=any_spec,
        scratch_shapes=[
            pltpu.VMEM((8, NA, 8, D), BF),
            pltpu.VMEM((8, NA, 8, D), BF),
            pltpu.VMEM((2, 4, DF, 512), BF),
            pltpu.VMEM((F, D), BF), pltpu.VMEM((F, D), BF),
            pltpu.VMEM((128, D), U32), pltpu.VMEM((128, D), U32),
            pltpu.VMEM((NA, 64, 128), U32), pltpu.VMEM((NA, 64, 128), U32),
            pltpu.VMEM((2, 64, 128), U32),
            pltpu.VMEM((8, F), F32), pltpu.VMEM((8, D), F32),
            pltpu.VMEM((8, 256, D), F32),
            pltpu.VMEM((NA, 3, 64, 128), U32),
            pltpu.VMEM((NA, 128, 256), F32), pltpu.VMEM((NA, 64, 128), F32),
            pltpu.VMEM((NA, 64, 256), F32), pltpu.VMEM((NA, 64, 256), F32),
            pltpu.VMEM((NA, 64, 128), F32), pltpu.VMEM((NA, 64, 128), F32),
            pltpu.VMEM((2, 2, 168, 128), U32),
            pltpu.VMEM((2, 256, D), BF),
            pltpu.VMEM((256, F), BF),
            pltpu.VMEM((4, 5, 4, 8, 8, 128), F32),
            pltpu.VMEM((2, 5, 4, 8, 8, 128), F32),
            pltpu.SemaphoreType.DMA((8,)), pltpu.SemaphoreType.DMA((8,)),
            pltpu.SemaphoreType.DMA((19,)), pltpu.SemaphoreType.DMA((8,)),
        ],
        compiler_params=pltpu.CompilerParams(vmem_limit_bytes=110 * 1024 * 1024),
    )(A_x.reshape(NA, 8, 8, D), A_w_r.T, A_w_i.T, B_w1.T, B_b1, B_w2, B_b2, *consts)
    return out.reshape(1, S, D)
```

```python
import math
import numpy as np
import jax
import jax.numpy as jnp
from jax import lax
import jax.experimental.pallas as pl
import jax.experimental.pallas.tpu as pltpu

S, D, F, DF = 2048, 640, 1728, 321
NA, NB = 32, 64
BF = jnp.bfloat16
F32 = jnp.float32
U32 = jnp.uint32

S1, S2 = math.sin(2 * math.pi / 5), math.sin(4 * math.pi / 5)
K5 = math.sqrt(5.0) / 4.0
R21 = S2 / S1
AORD = [4 * a2 + a1 for a1 in range(4) for a2 in range(8)]


def _fwd5(z):
    z0, z1, z2, z3, z4 = z
    s14 = z1 + z4; d14 = z1 - z4; s23 = z2 + z3; d23 = z2 - z3
    u = s14 + s23
    t0 = z0 + u
    m = z0 - 0.25 * u
    n = K5 * (s14 - s23)
    return t0, m + n, d14 + R21 * d23, m - n, R21 * d14 - d23


_GROUPS = {1: [(1, 6), (9, 4)], 2: [(7, 2), (3, 8)], 0: [(5, 10)]}


def _inv5k(q):
    q0, q1r, q1i, q2r, q2i = q
    u = q1r + q2r
    y0 = q0 + u
    m = q0 - 0.25 * u
    n = K5 * (q1r - q2r)
    a1 = m + n; a2 = m - n
    b1 = S1 * q1i + S2 * q2i
    b2 = S2 * q1i - S1 * q2i
    return y0, a1 - b1, a2 - b2, a2 + b2, a1 + b1


def _fwd5k(z):
    z0, z1, z2, z3, z4 = z
    s14 = z1 + z4; d14 = z1 - z4; s23 = z2 + z3; d23 = z2 - z3
    u = s14 + s23
    t0 = z0 + u
    m = z0 - 0.25 * u
    n = K5 * (s14 - s23)
    return t0, m + n, S1 * d14 + S2 * d23, m - n, S2 * d14 - S1 * d23


def _lane_plan():
    out = {}
    for cl, prs in _GROUPS.items():
        kd = []
        for (rh, rl) in prs:
            for m in range(32):
                kd += [rh + 10 * m, rl + 10 * m]
        out[cl] = np.array(kd, np.int64)
    return out[0], out[1], out[2]


def _build_consts():
    kd0, kd1, kd2 = _lane_plan()
    n = np.arange(D)
    eye = np.eye(D)

    def cs(kd):
        th = 2 * np.pi * np.outer(n, kd) / D
        return np.cos(th), np.sin(th)
    c0, s0 = cs(kd0); c1, s1 = cs(kd1); c2, s2 = cs(kd2)
    s0[:, kd0 == 320] = 0.0
    tiles = [eye[:, 128 * a:128 * (a + 1)] for a in range(5)]
    Ffull = np.concatenate([c0, -s0, c1, -s1, c2, -s2], axis=1)
    Fm = np.linalg.solve(np.concatenate(_fwd5(tiles), axis=1), Ffull)
    kap = lambda kd: np.where(kd == 320, 1.0, 2.0)
    Gfull = np.concatenate([(c0 * kap(kd0)).T, (-s0 * kap(kd0)).T, (c1 * kap(kd1)).T, (-s1 * kap(kd1)).T,
                            (c2 * kap(kd2)).T, (-s2 * kap(kd2)).T], axis=0) / (D * S)
    b = np.arange(64)
    kr = 16 * (b // 8) + 2 * (b % 8); ki = kr + 1
    pos = np.arange(64)
    psi = 2 * np.pi * np.outer(pos, b) / 64
    A0 = np.zeros((128, 128)); B0 = np.zeros((128, 128))
    A0[np.ix_(pos, kr)] = np.cos(psi); A0[np.ix_(pos, ki)] = np.sin(psi)
    A0[np.ix_(64 + pos, kr)] = -np.sin(psi); A0[np.ix_(64 + pos, ki)] = np.cos(psi)
    B0[np.ix_(pos, kr)] = -np.sin(psi); B0[np.ix_(pos, ki)] = np.cos(psi)
    B0[np.ix_(64 + pos, kr)] = -np.cos(psi); B0[np.ix_(64 + pos, ki)] = -np.sin(psi)
    TAB = np.stack([A0, B0]).astype(np.float32)
    phi = 2 * np.pi * np.outer(np.arange(NA), b) / S
    CS = np.zeros((2, NA, 128))
    CS[0][:, kr] = np.cos(phi); CS[0][:, ki] = np.cos(phi)
    CS[1][:, kr] = np.sin(phi); CS[1][:, ki] = np.sin(phi)
    CS = CS.astype(np.float32)
    Pm = np.zeros((128, 128))
    Pm[b, kr] = 1.0; Pm[64 + b, ki] = 1.0
    L = np.zeros((3, 128, 128))
    L[2] = Pm
    for par in range(2):
        for m in range(128):
            gam, j = m // 8, m % 8
            c = 2 * gam + ((j >= 4) if par == 0 else (j < 4))
            L[par, m, c + 32 * (j % 4)] = 1.0
    bf = lambda x: np.asarray(x, dtype=np.float32).astype(BF)
    sg = np.concatenate([np.ones(64), -np.ones(64)])
    FK = [Fm[0:128, 0:128]]
    for o in (128, 384):
        P = Fm[o:o + 128, o:o + 128]; Q = Fm[o + 128:o + 256, o:o + 128] / S1
        R = Fm[o:o + 128, o + 128:o + 256]; T = Fm[o + 128:o + 256, o + 128:o + 256] / S1
        assert np.abs(T + sg[None, :] * P).max() < 1e-9 and np.abs(R - sg[None, :] * Q).max() < 1e-9
        FK += [P, P + Q, P - Q]
    FK = np.concatenate(FK, axis=1)
    tiles = [eye[:, 128 * a:128 * (a + 1)] for a in range(5)]
    Gk = np.linalg.solve(np.concatenate(_inv5k(tiles), axis=1).T, Gfull.T).T
    GK = [Gk[0:128, 0:128]]
    for o in (128, 384):
        P = Gk[o:o + 128, o:o + 128]; Q = Gk[o + 128:o + 256, o:o + 128]
        R = Gk[o:o + 128, o + 128:o + 256]; T = Gk[o + 128:o + 256, o + 128:o + 256]
        Qt = sg[:, None] * Q; Tt = sg[:, None] * T
        assert np.abs(Tt - P).max() < 1e-12 and np.abs(Qt + R).max() < 1e-12
        GK += [P, P + R, R - P]
    GK = np.concatenate(GK, axis=1)
    def w32(a):
        u = np.asarray(a).view(np.uint16).astype(np.uint32)
        return np.ascontiguousarray(u[..., 0::2, :] | (u[..., 1::2, :] << 16))
    return dict(Fc=w32(bf(FK)), Gc=w32(bf(GK)), TAB=TAB, CS=CS, L=w32(bf(L)))


class _Cplx:
    @staticmethod
    def add(a, b): return (a[0] + b[0], a[1] + b[1])
    @staticmethod
    def sub(a, b): return (a[0] - b[0], a[1] - b[1])
    @staticmethod
    def addsubi(a, b):
        return (a[0] - b[1], a[1] + b[0]), (a[0] + b[1], a[1] - b[0])
    @staticmethod
    def muli(a, sg):
        return (-a[1], a[0]) if sg > 0 else (a[1], -a[0])
    @staticmethod
    def mul(a, c, s):
        if abs(abs(c) - abs(s)) < 1e-12:
            if s * c > 0:
                return (c * (a[0] - a[1]), c * (a[0] + a[1]))
            return (c * (a[0] + a[1]), c * (a[1] - a[0]))
        return (c * a[0] - s * a[1], c * a[1] + s * a[0])


def _fft(x, A, sign):
    N = len(x)
    if N == 1:
        return [x[0]]
    if N == 2:
        return [A.add(x[0], x[1]), A.sub(x[0], x[1])]
    E = _fft(x[0::2], A, sign); O1 = _fft(x[1::4], A, sign); O3 = _fft(x[3::4], A, sign)
    X = [None] * N
    for k in range(N // 4):
        t1, t3 = O1[k], O3[k]
        if k:
            a1 = sign * 2 * math.pi * k / N; a3 = 3 * a1
            t1 = A.mul(t1, math.cos(a1), math.sin(a1)); t3 = A.mul(t3, math.cos(a3), math.sin(a3))
        s = A.add(t1, t3); d = A.sub(t1, t3)
        X[k] = A.add(E[k], s); X[k + N // 2] = A.sub(E[k], s)
        p, m = A.addsubi(E[k + N // 4], d)
        if sign > 0:
            X[k + N // 4], X[k + 3 * N // 4] = p, m
        else:
            X[k + N // 4], X[k + 3 * N // 4] = m, p
    return X


def _tw(A, v, a1, c2, sign):
    n = (a1 * c2) % 32
    if n == 0:
        return v
    if n == 8:
        return A.muli(v, sign)
    ang = sign * 2 * math.pi * n / 32
    return A.mul(v, math.cos(ang), math.sin(ang))


def _dot(a, b):
    return jnp.dot(a, b, preferred_element_type=F32)


def _dot_nt(a, b):
    return lax.dot_general(a, b, (((1,), (1,)), ((), ())), preferred_element_type=F32)


def _gelu(h):
    inner = h * (0.7978845608028654 + (0.7978845608028654 * 0.044715) * (h * h))
    hh = 0.5 * h
    return hh + hh * jnp.tanh(inner)


def _run(gen):
    for _ in gen:
        pass


def _pk(v):
    return pltpu.bitcast(v, U32)


def _upk(w):
    return pltpu.bitcast(w, BF)


def _kernel(x_hbm, wr_hbm, wi_hbm, w1_hbm, b1_hbm, w2_hbm, b2_hbm,
            Fc_hbm, Gc_hbm, TAB_hbm, CS_hbm, L_hbm, z_hbm,
            o_hbm,
            XI, O, Wraw, w1_ref, w2_ref, Fc, Gc, Mf_ref, Mi_ref, L_ref, b1f, b2f, b1c,
            X, V, H12, H0, Wr12, Wi12, Wa0, Wb0, Wst, XN, G, Ys, Zs, b1_ref, b2_ref, z_ref, TAB, CS,
            sx, sw, sm, so, sb):
    lane = lax.broadcasted_iota(jnp.int32, (8, 128), 1)
    sub = lax.broadcasted_iota(jnp.int32, (8, 128), 0)
    lo8 = lane < 64
    sig8 = jnp.where(lo8, -1.0, 1.0).astype(F32)

    cx = [pltpu.make_async_copy(x_hbm.at[:, g], XI.at[g], sx.at[g]) for g in range(8)]
    cw = [pltpu.make_async_copy((wr_hbm, wi_hbm)[k].at[:, pl.ds(512 * q, 512)], Wraw.at[k, q], sw.at[2 * q + k])
          for q in range(4) for k in range(2)]
    cF = pltpu.make_async_copy(Fc_hbm, Fc, sm.at[0])
    cG = pltpu.make_async_copy(Gc_hbm, Gc, sm.at[1])
    cL = pltpu.make_async_copy(L_hbm, L_ref, sm.at[2])
    cT = pltpu.make_async_copy(TAB_hbm, TAB.at[pl.ds(0, 2)], sm.at[3])
    cC = pltpu.make_async_copy(CS_hbm, CS, sm.at[4])
    cw1 = [pltpu.make_async_copy(w1_hbm.at[pl.ds(a, n)], w1_ref.at[pl.ds(a, n)], sm.at[11 + i])
           for i, (a, n) in enumerate(((0, 640), (640, 512), (1152, 576)))]
    cw2 = [pltpu.make_async_copy(w2_hbm.at[:, pl.ds(128 * n, 128)], w2_ref.at[:, pl.ds(128 * n, 128)], sm.at[14 + n])
           for n in range(5)]
    cT.start(); cC.start(); cL.start(); cx[0].start(priority=1); cF.start(priority=1); cx[1].start(priority=1)

    cb = [pltpu.make_async_copy(b1_hbm, b1_ref, sb.at[0]), pltpu.make_async_copy(b2_hbm, b2_ref, sb.at[1]),
          pltpu.make_async_copy(z_hbm, z_ref, sb.at[2])]

    def bias_setup():
        for c in cb[0:2]:
            c.wait()
        b1f[...] = jnp.broadcast_to(b1_ref[...].astype(F32)[None, :], (8, F))
        b2f[...] = jnp.broadcast_to(b2_ref[...].astype(F32)[None, :], (8, D))
        b1c[...] = jnp.broadcast_to(b1f[:, 1664:F].T[:, 0:1], (64, 128))
    Fk = lambda i: _upk(Fc[:, 128 * i:128 * i + 128])
    Gk = lambda i: _upk(Gc[:, 128 * i:128 * i + 128])

    def wprep(q):
        lo4 = sub < 4
        for tp in range(2):
            outs = []
            for par in range(2):
                tl = 2 * tp + par
                Lm = _upk(L_ref[par])
                o = []
                for k in range(2):
                    Wst[k, par, 0:160, :] = _pk(Wraw[k, q, 0:320, 128 * tl:128 * tl + 128])
                    Wst[k, par, 160:161, :] = pltpu.bitcast(
                        Wraw[k, q, 320:321, 128 * tl:128 * tl + 128].astype(F32), U32) >> 16

                    def tile(cl):
                        ws = []
                        for (rh, rl) in _GROUPS[cl]:
                            hi = Wst[k, par, pl.ds(rh // 2, 32, stride=5), :]
                            lo = Wst[k, par, pl.ds(rl // 2, 32, stride=5), :]
                            ws.append((hi >> 16) | (lo << 16))
                        return jnp.concatenate(ws, axis=0) if len(ws) > 1 else ws[0]
                    t1 = _dot_nt(Lm, _upk(tile(1)))
                    t2 = _dot_nt(Lm, _upk(tile(2)))
                    w0 = tile(0)
                    w0 = jnp.concatenate([w0, w0] if k == 0 else [w0 ^ jnp.uint32(0x80008000), w0], axis=0)
                    t0 = _dot_nt(Lm, _upk(w0))
                    o += [t1, t2, t0]
                outs.append(o)
                yield
            G8 = 8 * (2 * q + tp)
            dst = [(Wr12, 0), (Wr12, 128), (Wa0, 0), (Wi12, 0), (Wi12, 128), (Wb0, 0)]
            for ti in range(6):
                ref, l0 = dst[ti]
                for gam in range(16):
                    A_ = outs[0][ti][8 * gam:8 * gam + 8]; B_ = outs[1][ti][8 * gam:8 * gam + 8]
                    ref[2 * gam, G8:G8 + 8, l0:l0 + 128] = jnp.where(lo4, A_, B_)
                    ref[2 * gam + 1, G8:G8 + 8, l0:l0 + 128] = jnp.where(lo4, B_, A_)
            yield

    sigp = -sig8
    sigp64 = jnp.where(lax.broadcasted_iota(jnp.int32, (64, 128), 1) < 64, 1.0, -1.0).astype(F32)

    zf = {}

    def gate(val, fake):
        if fake is None:
            return val
        return jnp.where(zf['v'], pltpu.bitcast(fake, val.dtype), val)

    def orall(vs):
        vs = [pltpu.bitcast(v, U32) for v in vs]
        while len(vs) > 1:
            vs = [vs[i] | vs[i + 1] if i + 1 < len(vs) else vs[i] for i in range(0, len(vs), 2)]
        return vs[0]

    def vregs(v):
        return [v[8 * i:8 * i + 8, 128 * n:128 * n + 128] for i in range(v.shape[0] // 8) for n in range(v.shape[1] // 128)]

    def gate0(x, fake):
        if fake is None:
            return x
        top = jnp.concatenate([gate(x[0:8, 0:128], fake), x[0:8, 128:]], axis=1)
        return jnp.concatenate([top, x[8:]], axis=0)

    def jp(v):
        return pltpu.roll(v, 64, 1) * sigp

    def rowsum(x):
        return jnp.sum(x, axis=1, keepdims=True)

    def xin(g, a1):
        return jnp.concatenate([XI[g, AORD[8 * a1 + a2]].astype(F32) for a2 in range(8)], axis=0)

    def stC1(g, slot, first=False, chain=False):
        fake = None
        for a1 in range(4):
            r0 = 64 * a1
            x = xin(g, a1) if first else X[g, r0:r0 + 64, :]
            x = gate0(x, fake)
            outs = []
            t0, t1r, t1i, t2r, t2i = _fwd5k([x[:, 128 * a:128 * (a + 1)] for a in range(5)])
            k1 = _dot((t1r - t1i).astype(BF), Fk(1)); m1 = _dot(t1i.astype(BF), Fk(2)); n1 = _dot(t1r.astype(BF), Fk(3))
            k2 = _dot((t2r - t2i).astype(BF), Fk(4)); m2 = _dot(t2i.astype(BF), Fk(5)); n2 = _dot(t2r.astype(BF), Fk(6))
            p = (t1r * t1r + t2r * t2r) + (t1i * t1i + t2i * t2i)
            m5 = rowsum(t0) * (1.0 / 128)
            yield
            t0c = t0 - m5
            U0 = _dot(t0c.astype(BF), Fk(0))
            v = rowsum(2.0 * p + t0c * t0c)
            yield
            rs = jnp.exp2(-0.5 * jnp.log2(v * (1.0 / (5 * D)) + 1e-5))
            rss = rs * sigp64
            U0 = U0 * rs
            U1 = jnp.concatenate([(k1 + m1) * rs, (k1 - n1) * rss], axis=1)
            U2 = jnp.concatenate([(k2 + m2) * rs, (k2 - n2) * rss], axis=1)
            x0 = [(U0[8 * a2:8 * a2 + 8], jp(U0[8 * a2:8 * a2 + 8])) for a2 in range(8)]
            for cl, Uc in ((1, U1), (2, U2)):
                xs = [(Uc[8 * a2:8 * a2 + 8, :128], Uc[8 * a2:8 * a2 + 8, 128:]) for a2 in range(8)]
                Y = _fft(xs, _Cplx, -1)
                for c2 in range(8):
                    w = _tw(_Cplx, Y[c2], a1, c2, -1)
                    Ys[slot, 2 * cl - 1, a1, c2] = w[0]; Ys[slot, 2 * cl, a1, c2] = w[1]
                    outs += [w[0], w[1]]
                yield
            Y = _fft(x0, _Cplx, -1)
            for c2 in range(8):
                w = _tw(_Cplx, Y[c2], a1, c2, -1)[0]
                Ys[slot, 0, a1, c2] = w
                outs.append(w)
            if chain:
                fake = orall(outs)
            yield

    def stC2(g, slot, chain=False):
        r0 = pl.multiple_of(8 * g, 8)
        fake = None
        for c2 in range(8):
            y0 = [Ys[slot, 0, a1, c2] for a1 in range(4)]
            y0[0] = gate(y0[0], fake)
            x0 = [(y, jp(y)) for y in y0]
            outs = []
            for cl in (1, 2, 0):
                if cl:
                    xs = [(Ys[slot, 2 * cl - 1, a1, c2], Ys[slot, 2 * cl, a1, c2]) for a1 in range(4)]
                    xs[0] = (gate(xs[0][0], fake), gate(xs[0][1], fake))
                else:
                    xs = x0
                Xo = _fft(xs, _Cplx, -1)
                for c1 in range(4):
                    w = pltpu.pack_elementwise([Xo[c1][0], Xo[c1][1]], packed_dtype=BF)
                    V[c2 + 8 * c1, cl, pl.ds(r0, 8), :] = w
                    outs.append(w)
            if chain:
                fake = orall(outs)
            yield

    def stA1(g, slot, chain=False):
        r0 = pl.multiple_of(8 * g, 8)
        fake = None
        for c2 in range(8):
            h0 = [H0[c2 + 8 * c1, pl.ds(r0, 8), :] for c1 in range(4)]
            h0[0] = gate(h0[0], fake)
            x0 = [(h, jp(h)) for h in h0]
            outs = []
            for cl in (1, 2):
                l0 = 128 * (cl - 1)
                xs = [(H12[c2 + 8 * c1, pl.ds(r0, 8), l0:l0 + 128], H12[c2 + 8 * c1, pl.ds(64 + r0, 8), l0:l0 + 128])
                      for c1 in range(4)]
                xs[0] = (gate(xs[0][0], fake), gate(xs[0][1], fake))
                Zq = _fft(xs, _Cplx, +1)
                for a1 in range(4):
                    v = _tw(_Cplx, Zq[a1], a1, c2, +1)
                    Zs[slot, 2 * cl - 1, a1, c2] = v[0]; Zs[slot, 2 * cl, a1, c2] = v[1]
                    outs += [v[0], v[1]]
            Zq = _fft(x0, _Cplx, +1)
            for a1 in range(4):
                v = _tw(_Cplx, Zq[a1], a1, c2, +1)[0]
                Zs[slot, 0, a1, c2] = v
                outs.append(v)
            if chain:
                fake = orall(outs)
            yield

    def stA2(g, slot, xslot, first=False, chain=False):
        fake = None
        for a1 in range(4):
            r0 = 64 * a1
            z0 = [Zs[slot, 0, a1, c2] for c2 in range(8)]
            z0[0] = gate(z0[0], fake)
            x0 = [(z, jp(z)) for z in z0]
            tl = [None] * 5
            for cl in (1, 2):
                Vo = _fft([(Zs[slot, 2 * cl - 1, a1, c2], Zs[slot, 2 * cl, a1, c2]) for c2 in range(8)], _Cplx, +1)
                for ri in range(2):
                    tl[2 * cl - 1 + ri] = jnp.concatenate([o[ri] for o in Vo], axis=0)
            Vo = _fft(x0, _Cplx, +1)
            tl[0] = jnp.concatenate([o[0] for o in Vo], axis=0)
            qs = []
            for cl in (1, 2):
                vr = tl[2 * cl - 1]; vi = tl[2 * cl] * sigp64
                o = 3 * cl - 2
                mm = _dot((vr + vi).astype(BF), Gk(o))
                qs.append((mm, _dot(vi.astype(BF), Gk(o + 1)), _dot(vr.astype(BF), Gk(o + 2))))
            q0 = _dot(tl[0].astype(BF), Gk(0))
            yield
            ys = _inv5k([q0, qs[0][0] - qs[0][1], qs[0][0] + qs[0][2], qs[1][0] - qs[1][1], qs[1][0] + qs[1][2]])
            x1 = (xin(g, a1) if first else X[g, r0:r0 + 64, :]) + jnp.concatenate(ys, axis=1)
            X[g, r0:r0 + 64, :] = x1
            m = rowsum(x1) * (1.0 / D)
            yield
            d = X[g, r0:r0 + 64, :] - m
            v = rowsum(d * d)
            yield
            rs = jnp.exp2(-0.5 * jnp.log2(v * (1.0 / D) + 1e-5))
            xn = (X[g, r0:r0 + 64, :] - m) * rs
            XN[xslot, r0:r0 + 64, :] = xn.astype(BF)
            if chain:
                fake = orall(vregs(rs + jnp.zeros((64, 128), F32)))
            yield

    def stB1(g, slot):
        def tchunk():
            hT = _dot_nt(w1_ref[1664:F, :], XN[slot])
            for hh in range(2):
                gT = _gelu(hT[:, 128 * hh:128 * hh + 128] + b1c[...])
                G[128 * hh:128 * hh + 128, 1664:F] = gT.T.astype(BF)
        tpos = 13
        for j in range(14):
            if j == tpos:
                tchunk()
            else:
                jj = j if j < tpos else j - 1
                n0, n1 = 128 * jj, 128 * jj + 128
                h = _dot_nt(XN[slot], w1_ref[n0:n1, :]) + b1f[0:1, n0:n1]
                G[:, n0:n1] = _gelu(h).astype(BF)
            yield

    def stB1s(g, slot):
        for rh in range(2):
            r0 = 128 * rh
            for j in range(13):
                n0, n1 = 128 * j, 128 * j + 128
                h = _dot_nt(XN[slot, r0:r0 + 128, :], w1_ref[n0:n1, :]) + b1f[0:1, n0:n1]
                G[r0:r0 + 128, n0:n1] = _gelu(h).astype(BF)
                yield
        hT = _dot_nt(w1_ref[1664:F, :], XN[slot])
        for hh in range(2):
            gT = _gelu(hT[:, 128 * hh:128 * hh + 128] + b1c[...])
            G[128 * hh:128 * hh + 128, 1664:F] = gT.T.astype(BF)
        yield

    def out_col(g, n):
        return pltpu.make_async_copy(O.at[g, :, :, pl.ds(128 * n, 128)], o_hbm.at[:, g, :, pl.ds(128 * n, 128)], so.at[8 + n])

    def stB2(g, slot, last=False, tail=False):
        for n, rh in [(n, rh) for n in range(5) for rh in range(2)]:
            r0 = 128 * rh
            o = _dot(G[r0:r0 + 128, :], w2_ref[:, 128 * n:128 * n + 128]) + b2f[0:1, 128 * n:128 * n + 128]
            x2 = X[g, r0:r0 + 128, 128 * n:128 * n + 128] + o
            if last:
                for pp in range(16):
                    O[g, AORD[16 * rh + pp], :, 128 * n:128 * n + 128] = x2[8 * pp:8 * pp + 8].astype(BF)
            else:
                X[g, r0:r0 + 128, 128 * n:128 * n + 128] = x2
            if tail and rh == 1:
                out_col(g, n).start()
            yield

    def interleave(main, fillers):
        live = [[f, q, 0.0] for f, q in fillers]
        for _ in main:
            nxt = []
            for e in live:
                e[2] += e[1]
                alive = True
                while e[2] >= 1.0 - 1e-9:
                    e[2] -= 1.0
                    try:
                        next(e[0])
                    except StopIteration:
                        alive = False
                        break
                if alive:
                    nxt.append(e)
            live = nxt
        for e in live:
            _run(e[0])

    sig64 = jnp.where(lax.broadcasted_iota(jnp.int32, (64, 128), 1) < 64, 1.0, -1.0).astype(F32)

    def s_phase(first):
        GP = 2
        NG = NA // GP
        Zq = {}; Y = {}; Hh = {}
        cs = lambda p: [GP * p + u for u in range(GP)] if 0 <= p < NG else []
        for i in range(NG + 3):
            for c in cs(i - 3):
                h12, h0 = Hh.pop(c)
                H12[c] = h12; H0[c] = h0
            a = {}; b = {}
            for c in cs(i - 2):
                a[c] = _dot(Mi_ref[c], Y[c][0])
            for c in cs(i):
                v12 = jnp.concatenate([_upk(V[c, 1]), _upk(V[c, 2])], axis=1)
                b[c] = _dot(Mf_ref[c], v12)
            for c in cs(i - 2):
                Hh[c] = (a[c], _dot(Mi_ref[c, 0:64], Y.pop(c)[1]))
            for c in cs(i):
                Zq[c] = (b[c], _dot(Mf_ref[c, 0:64], _upk(V[c, 0])))
            for c in cs(i - 1):
                z12, z0 = Zq.pop(c)
                Zr, Zi = z12[0:64], z12[64:128]
                wr = Wr12[c]; wi = Wi12[c]
                y12 = jnp.concatenate([Zr * wr - Zi * wi, Zr * wi + Zi * wr], axis=0).astype(BF)
                y0 = z0 * Wa0[c] + pltpu.roll(z0, 64, 1) * Wb0[c]
                st = jnp.concatenate([y0, pltpu.roll(y0, 64, 1) * sig64], axis=0).astype(BF)
                Y[c] = (y12, st)

    def gen_m():
        cT.wait(); cC.wait(); cL.wait()
        for t in range(2):
            v = TAB[t]
            TAB[2 + t] = jnp.concatenate(
                [v[8 * i + 4 * h:8 * i + 4 * h + 4] for i in range(16) for h in (1, 0)], axis=0)
        Pm = _upk(L_ref[2])
        for c in range(NA):
            o = 2 * (c % 2)
            m = TAB[o] * CS[0, c:c + 1, :] + TAB[o + 1] * CS[1, c:c + 1, :]
            mb = m.astype(BF)
            Mf_ref[c] = mb
            Mi_ref[c] = _dot_nt(Pm, mb).astype(BF)

    with jax.named_scope('ph1'):
        P1 = dict(priority=1)

        def pair(g):
            interleave(stC1(g, g % 4, True), [(stC1(g + 1, (g + 1) % 4, True), 1.0)])
            _run(stC2(g - 2, (g - 2) % 4)); _run(stC2(g - 1, (g - 1) % 4))
        gen_m()
        cx[0].wait()
        for g in range(2, 8):
            cx[g].start(**P1)
        cF.wait(); cx[1].wait()
        for c in cw:
            c.start(**P1)
        for c in cb:
            c.start(**P1)
        interleave(stC1(0, 0, True), [(stC1(1, 1, True), 1.0)])
        for g in (2, 4):
            cx[g].wait(); cx[g + 1].wait()
            if g == 4:
                cG.start(**P1)
                cw1[0].start(**P1)
            pair(g)
        cx[6].wait(); cx[7].wait()
        cw1[1].start(**P1); cw1[2].start(**P1)
        pair(6)
        cw[0].wait(); cw[1].wait(); cw[2].wait(); cw[3].wait(); cb[2].wait()
        zf['v'] = z_ref[0] == 1
        for c_ in cw2[0:2]:
            c_.start(**P1)
        w01 = (y for gen in (wprep(0), wprep(1)) for y in gen)
        interleave(w01, [(stC2(6, 2, True), 0.7), (stC2(7, 3, True), 0.7)])
        cw[4].wait(); cw[5].wait()
        for c_ in cw2[2:5]:
            c_.start(**P1)
        bias_setup()
        _run(wprep(2))
    with jax.named_scope('s1'):
        cw[6].wait(); cw[7].wait(); cG.wait()
        _run(wprep(3))
        s_phase(True)

    def run_plan(mains, fillers):
        i = 0
        for mg in mains:
            for _ in mg:
                for f, plan in fillers:
                    for _ in range(plan[i] if i < len(plan) else 0):
                        try:
                            next(f)
                        except StopIteration:
                            pass
                i += 1
        for f, plan in fillers:
            _run(f)

    def spread(n, lo, hi, tot=24):
        out = [0] * tot
        for i in range(n):
            out[lo + (i * (hi - lo)) // n] += 1
        return out

    def out_copy(g):
        return pltpu.make_async_copy(O.at[g], o_hbm.at[:, g], so.at[g])

    def mlp_phase(last):
        first = not last
        if first:
            for c in cw1:
                c.wait()

        def body0_early():
            _run(stA1(0, 0))
            gA2 = stA2(0, 0, 0, first)
            for _ in range(8):
                next(gA2)
            nq = 27
            e0 = 6
            run_plan([stB1s(0, 0)], [(gA2, spread(8, 0, e0, nq)), (stA1(1, 0, True), spread(8, e0 + 2, nq, nq))])
            if first:
                for c in cw2:
                    c.wait()
            run_plan([stB2(0, 0, last)], [(stA2(1, 0, 1, first, True), spread(16, 0, 10, 10))])
            if last:
                out_copy(0).start()

        def body(g, hasC, hasA, tail=False):
            fl = []
            if hasC:
                fl.append((stC1(g - 1, 0, False, True), spread(20, 0, 14)))
                fl.append((stC2(g - 1, 0, True), spread(8, 14, 24)))
            if hasA:
                fl.append((stA1(g + 1, 0, True), spread(8, 0, 14)))
                fl.append((stA2(g + 1, 0, (g + 1) % 2, first, True), spread(16, 14, 24)))
            run_plan([stB1(g, g % 2), stB2(g, g % 2, last, tail)], fl)
            if last and not tail:
                out_copy(g).start()
        body0_early()
        if last:
            lax.fori_loop(1, 7, lambda g, c: (body(g, False, True), c)[1], 0)
            body(7, False, False, tail=True)
        else:
            lax.fori_loop(1, 7, lambda g, c: (body(g, True, True), c)[1], 0)
            body(7, True, False)
            _run(stC1(7, 0))
            _run(stC2(7, 0))

    with jax.named_scope('ph2'):
        mlp_phase(False)
    with jax.named_scope('s2'):
        s_phase(False)
    with jax.named_scope('ph3'):
        mlp_phase(True)
    for g in range(7):
        out_copy(g).wait()
    for n in range(5):
        out_col(7, n).wait()


_K = None


@jax.jit
def pallas_interleave_layers__spectral_gfnet__dense_activation_gelu__prompt_kernel(A_x, A_w_r, A_w_i, B_x, B_w1, B_b1, B_w2, B_b2):
    global _K
    if _K is None:
        _K = _build_consts()
    K = _K
    consts = [K[n] for n in ('Fc', 'Gc', 'TAB', 'CS', 'L')]
    any_spec = pl.BlockSpec(memory_space=pl.ANY)
    out = pl.pallas_call(
        _kernel,
        out_shape=jax.ShapeDtypeStruct((NA, 8, 8, D), BF),
        in_specs=[any_spec] * 13,
        out_specs=any_spec,
        scratch_shapes=[
            pltpu.VMEM((8, NA, 8, D), BF),
            pltpu.VMEM((8, NA, 8, D), BF),
            pltpu.VMEM((2, 4, DF, 512), BF),
            pltpu.VMEM((F, D), BF), pltpu.VMEM((F, D), BF),
            pltpu.VMEM((64, 896), U32), pltpu.VMEM((64, 896), U32),
            pltpu.VMEM((NA, 128, 128), BF), pltpu.VMEM((NA, 128, 128), BF),
            pltpu.VMEM((3, 64, 128), U32),
            pltpu.VMEM((8, F), F32), pltpu.VMEM((8, D), F32), pltpu.VMEM((64, 128), F32),
            pltpu.VMEM((8, 256, D), F32),
            pltpu.VMEM((NA, 3, 64, 128), U32),
            pltpu.VMEM((NA, 128, 256), F32), pltpu.VMEM((NA, 64, 128), F32),
            pltpu.VMEM((NA, 64, 256), F32), pltpu.VMEM((NA, 64, 256), F32),
            pltpu.VMEM((NA, 64, 128), F32), pltpu.VMEM((NA, 64, 128), F32),
            pltpu.VMEM((2, 2, 168, 128), U32),
            pltpu.VMEM((2, 256, D), BF),
            pltpu.VMEM((256, F), BF),
            pltpu.VMEM((4, 5, 4, 8, 8, 128), F32),
            pltpu.VMEM((2, 5, 4, 8, 8, 128), F32),
            pltpu.VMEM((F,), BF), pltpu.VMEM((D,), BF), pltpu.SMEM((4,), jnp.int32),
            pltpu.VMEM((4, 128, 128), F32), pltpu.VMEM((2, NA, 128), F32),
            pltpu.SemaphoreType.DMA((8,)), pltpu.SemaphoreType.DMA((8,)),
            pltpu.SemaphoreType.DMA((19,)), pltpu.SemaphoreType.DMA((13,)), pltpu.SemaphoreType.DMA((3,)),
        ],
        compiler_params=pltpu.CompilerParams(vmem_limit_bytes=110 * 1024 * 1024),
    )(A_x.reshape(NA, 8, 8, D), A_w_r.T, A_w_i.T, B_w1.T, B_b1, B_w2, B_b2, *consts, np.array([7, 3, 5, 2], dtype=np.int32))
    return out.reshape(1, S, D)
```

```python
import math
import numpy as np
import jax
import jax.numpy as jnp
from jax import lax
import jax.experimental.pallas as pl
import jax.experimental.pallas.tpu as pltpu

S, D, F, DF = 2048, 640, 1728, 321
NA, NB = 32, 64
BF = jnp.bfloat16
F32 = jnp.float32
U32 = jnp.uint32

S1, S2 = math.sin(2 * math.pi / 5), math.sin(4 * math.pi / 5)
K5 = math.sqrt(5.0) / 4.0
R21 = S2 / S1
AORD = [4 * a2 + a1 for a1 in range(4) for a2 in range(8)]


def _fwd5(z):
    z0, z1, z2, z3, z4 = z
    s14 = z1 + z4; d14 = z1 - z4; s23 = z2 + z3; d23 = z2 - z3
    u = s14 + s23
    t0 = z0 + u
    m = z0 - 0.25 * u
    n = K5 * (s14 - s23)
    return t0, m + n, d14 + R21 * d23, m - n, R21 * d14 - d23


_GROUPS = {1: [(6, 4), (1, 9)], 2: [(2, 8), (7, 3)], 0: [(5, 10)]}


def _inv5k(q):
    q0, q1r, q1i, q2r, q2i = q
    u = q1r + q2r
    y0 = q0 + u
    m = q0 - 0.25 * u
    n = K5 * (q1r - q2r)
    a1 = m + n; a2 = m - n
    b1 = S1 * q1i + S2 * q2i
    b2 = S2 * q1i - S1 * q2i
    return y0, a1 - b1, a2 - b2, a2 + b2, a1 + b1


def _fwd5k(z):
    z0, z1, z2, z3, z4 = z
    s14 = z1 + z4; d14 = z1 - z4; s23 = z2 + z3; d23 = z2 - z3
    u = s14 + s23
    t0 = z0 + u
    m = z0 - 0.25 * u
    n = K5 * (s14 - s23)
    return t0, m + n, S1 * d14 + S2 * d23, m - n, S2 * d14 - S1 * d23


def _lane_plan():
    out = {}
    for cl, prs in _GROUPS.items():
        kd = []
        for (rh, rl) in prs:
            for m in range(32):
                kd += [rh + 10 * m, rl + 10 * m]
        out[cl] = np.array(kd, np.int64)
    return out[0], out[1], out[2]


def _build_consts():
    kd0, kd1, kd2 = _lane_plan()
    n = np.arange(D)
    eye = np.eye(D)

    def cs(kd):
        th = 2 * np.pi * np.outer(n, kd) / D
        return np.cos(th), np.sin(th)
    c0, s0 = cs(kd0); c1, s1 = cs(kd1); c2, s2 = cs(kd2)
    s0[:, kd0 == 320] = 0.0
    tiles = [eye[:, 128 * a:128 * (a + 1)] for a in range(5)]
    Ffull = np.concatenate([c0, -s0, c1, -s1, c2, -s2], axis=1)
    Fm = np.linalg.solve(np.concatenate(_fwd5(tiles), axis=1), Ffull)
    kap = lambda kd: np.where(kd == 320, 1.0, 2.0)
    Gfull = np.concatenate([(c0 * kap(kd0)).T, (-s0 * kap(kd0)).T, (c1 * kap(kd1)).T, (-s1 * kap(kd1)).T,
                            (c2 * kap(kd2)).T, (-s2 * kap(kd2)).T], axis=0) / (D * S)
    b = np.arange(64)
    kr = 16 * (b // 8) + 2 * (b % 8); ki = kr + 1
    pos = np.arange(64)
    psi = 2 * np.pi * np.outer(pos, b) / 64
    A0 = np.zeros((128, 128)); B0 = np.zeros((128, 128))
    A0[np.ix_(pos, kr)] = np.cos(psi); A0[np.ix_(pos, ki)] = np.sin(psi)
    A0[np.ix_(64 + pos, kr)] = -np.sin(psi); A0[np.ix_(64 + pos, ki)] = np.cos(psi)
    B0[np.ix_(pos, kr)] = -np.sin(psi); B0[np.ix_(pos, ki)] = np.cos(psi)
    B0[np.ix_(64 + pos, kr)] = -np.cos(psi); B0[np.ix_(64 + pos, ki)] = -np.sin(psi)
    TAB = np.stack([A0, B0]).astype(np.float32)
    phi = 2 * np.pi * np.outer(np.arange(NA), b) / S
    CS = np.zeros((2, NA, 128))
    CS[0][:, kr] = np.cos(phi); CS[0][:, ki] = np.cos(phi)
    CS[1][:, kr] = np.sin(phi); CS[1][:, ki] = np.sin(phi)
    CS = CS.astype(np.float32)
    Pm = np.zeros((128, 128))
    Pm[b, kr] = 1.0; Pm[64 + b, ki] = 1.0
    L = np.zeros((3, 128, 128))
    L[2] = Pm
    for par in range(2):
        for m in range(128):
            gam, j = m // 8, m % 8
            c = 2 * gam + ((j >= 4) if par == 0 else (j < 4))
            L[par, m, c + 32 * (j % 4)] = 1.0
    bf = lambda x: np.asarray(x, dtype=np.float32).astype(BF)
    sg1 = np.where(np.isin(kd1 % 10, (1, 6)), 1.0, -1.0)
    assert np.array_equal(sg1, np.where(np.isin(kd2 % 10, (2, 7)), 1.0, -1.0)) and np.array_equal(sg1, np.tile([1.0, -1.0], 64))
    sg = sg1
    FK = [Fm[0:128, 0:128]]
    for o in (128, 384):
        P = Fm[o:o + 128, o:o + 128]; Q = Fm[o + 128:o + 256, o:o + 128] / S1
        R = Fm[o:o + 128, o + 128:o + 256]; T = Fm[o + 128:o + 256, o + 128:o + 256] / S1
        assert np.abs(T + sg[None, :] * P).max() < 1e-9 and np.abs(R - sg[None, :] * Q).max() < 1e-9
        FK += [P, P + Q, P - Q]
    lo = (np.arange(128) < 64)[None, :]
    sel = lambda a, b: np.where(lo, a, b)
    rol = lambda a: np.roll(a, 64, axis=1)

    def blocks(M):
        out = []
        for i in range(5):
            for j in range(5):
                blk = M[128 * i:128 * i + 128, 128 * j:128 * j + 128]
                if i == j:
                    out.append(blk)
                else:
                    assert np.abs(blk).max() < 1e-9 * np.abs(M).max(), (i, j, np.abs(blk).max())
        return out
    t0, t1r, t1i, t2r, t2i = _fwd5k([sel(tiles[a], tiles[(a + 2) % 5]) for a in range(5)])
    pre = [t0]
    for R, I in ((t1r, t1i), (t2r, t2i)):
        w2, rw = sel(R, I), rol(sel(I, R))
        pre += [w2 + rw, w2 - rw]
    post = [tiles[0]]
    for i in (1, 3):
        post += [sel(tiles[i], tiles[i + 1]), rol(sel(tiles[i + 1], tiles[i]))]
    F5 = blocks(np.linalg.solve(np.concatenate(pre, axis=1), Ffull) @ np.linalg.inv(np.concatenate(post, axis=1)))
    assert np.abs(F5[0] - FK[0]).max() < 1e-9
    FK = np.concatenate(FK + F5[1:], axis=1)
    pre = [tiles[0]]
    for i in (1, 3):
        y = rol(tiles[i + 1])
        pre += [sel(tiles[i], y), sel(y, tiles[i])]
    q = [tiles[0]]
    for i in (1, 3):
        y, y2 = rol(tiles[i] + tiles[i + 1]), tiles[i] - tiles[i + 1]
        q += [sel(y2, y), sel(y, y2)]
    zz = _inv5k(q)
    post = [sel(zz[a], zz[(a + 3) % 5]) for a in range(5)]
    GK = blocks(np.linalg.solve(np.concatenate(pre, axis=1), Gfull) @ np.linalg.inv(np.concatenate(post, axis=1)))
    Gk = np.linalg.solve(np.concatenate(_inv5k(tiles), axis=1).T, Gfull.T).T
    assert np.abs(Gk[0:128, 0:128] - GK[0]).max() < 1e-12
    for o in (128, 384):
        P = Gk[o:o + 128, o:o + 128]; Q = Gk[o + 128:o + 256, o:o + 128]
        R = Gk[o:o + 128, o + 128:o + 256]; T = Gk[o + 128:o + 256, o + 128:o + 256]
        Qt = sg[:, None] * Q; Tt = sg[:, None] * T
        assert np.abs(Tt - P).max() < 1e-12 and np.abs(Qt + R).max() < 1e-12
        GK += [P, P + R, R - P]
    GK = np.concatenate(GK, axis=1)
    def w32(a):
        u = np.asarray(a).view(np.uint16).astype(np.uint32)
        return np.ascontiguousarray(u[..., 0::2, :] | (u[..., 1::2, :] << 16))
    return dict(Fc=w32(bf(FK)), Gc=w32(bf(GK)), TAB=TAB, CS=CS, L=w32(bf(L)))


class _Cplx:
    @staticmethod
    def add(a, b): return (a[0] + b[0], a[1] + b[1])
    @staticmethod
    def sub(a, b): return (a[0] - b[0], a[1] - b[1])
    @staticmethod
    def addsubi(a, b):
        return (a[0] - b[1], a[1] + b[0]), (a[0] + b[1], a[1] - b[0])
    @staticmethod
    def muli(a, sg):
        return (-a[1], a[0]) if sg > 0 else (a[1], -a[0])
    @staticmethod
    def mul(a, c, s):
        if abs(abs(c) - abs(s)) < 1e-12:
            if s * c > 0:
                return (c * (a[0] - a[1]), c * (a[0] + a[1]))
            return (c * (a[0] + a[1]), c * (a[1] - a[0]))
        return (c * a[0] - s * a[1], c * a[1] + s * a[0])


def _fft(x, A, sign):
    N = len(x)
    if N == 1:
        return [x[0]]
    if N == 2:
        return [A.add(x[0], x[1]), A.sub(x[0], x[1])]
    E = _fft(x[0::2], A, sign); O1 = _fft(x[1::4], A, sign); O3 = _fft(x[3::4], A, sign)
    X = [None] * N
    for k in range(N // 4):
        t1, t3 = O1[k], O3[k]
        if k:
            a1 = sign * 2 * math.pi * k / N; a3 = 3 * a1
            t1 = A.mul(t1, math.cos(a1), math.sin(a1)); t3 = A.mul(t3, math.cos(a3), math.sin(a3))
        s = A.add(t1, t3); d = A.sub(t1, t3)
        X[k] = A.add(E[k], s); X[k + N // 2] = A.sub(E[k], s)
        p, m = A.addsubi(E[k + N // 4], d)
        if sign > 0:
            X[k + N // 4], X[k + 3 * N // 4] = p, m
        else:
            X[k + N // 4], X[k + 3 * N // 4] = m, p
    return X


def _tw(A, v, a1, c2, sign):
    n = (a1 * c2) % 32
    if n == 0:
        return v
    if n == 8:
        return A.muli(v, sign)
    ang = sign * 2 * math.pi * n / 32
    return A.mul(v, math.cos(ang), math.sin(ang))


def _dot(a, b):
    return jnp.dot(a, b, preferred_element_type=F32)


def _dot_nt(a, b):
    return lax.dot_general(a, b, (((1,), (1,)), ((), ())), preferred_element_type=F32)


def _gelu(h):
    inner = h * (0.7978845608028654 + (0.7978845608028654 * 0.044715) * (h * h))
    hh = 0.5 * h
    return hh + hh * jnp.tanh(inner)


def _run(gen):
    for _ in gen:
        pass


def _pk(v):
    return pltpu.bitcast(v, U32)


def _upk(w):
    return pltpu.bitcast(w, BF)


def _kernel(x_hbm, wr_hbm, wi_hbm, w1_hbm, b1_hbm, w2_hbm, b2_hbm,
            Fc_hbm, Gc_hbm, TAB_hbm, CS_hbm, L_hbm, z_hbm,
            o_hbm,
            XI, O, Wraw, w1_ref, w2_ref, Fc, Gc, Mf_ref, Mi_ref, L_ref, b1f, b2f, b1c,
            X, V, H12, H0, Wr12, Wi12, Wa0, Wb0, Wst, XN, G, Ys, Zs, b1_ref, b2_ref, z_ref, TAB, CS,
            sx, sw, sm, so, sb):
    lane = lax.broadcasted_iota(jnp.int32, (8, 128), 1)
    sub = lax.broadcasted_iota(jnp.int32, (8, 128), 0)
    lo8 = lane < 64
    sig8 = jnp.where(lo8, -1.0, 1.0).astype(F32)

    cx = [pltpu.make_async_copy(x_hbm.at[:, g], XI.at[g], sx.at[g]) for g in range(8)]
    cw = [pltpu.make_async_copy((wr_hbm, wi_hbm)[k].at[:, pl.ds(512 * q, 512)], Wraw.at[k, q], sw.at[2 * q + k])
          for q in range(4) for k in range(2)]
    cF = pltpu.make_async_copy(Fc_hbm, Fc, sm.at[0])
    cG = pltpu.make_async_copy(Gc_hbm, Gc, sm.at[1])
    cL = pltpu.make_async_copy(L_hbm, L_ref, sm.at[2])
    cT = pltpu.make_async_copy(TAB_hbm, TAB.at[pl.ds(0, 2)], sm.at[3])
    cC = pltpu.make_async_copy(CS_hbm, CS, sm.at[4])
    cw1 = [pltpu.make_async_copy(w1_hbm.at[pl.ds(a, n)], w1_ref.at[pl.ds(a, n)], sm.at[11 + i])
           for i, (a, n) in enumerate(((0, 640), (640, 512), (1152, 576)))]
    cw2 = [pltpu.make_async_copy(w2_hbm.at[:, pl.ds(128 * n, 128)], w2_ref.at[:, pl.ds(128 * n, 128)], sm.at[14 + n])
           for n in range(5)]
    cT.start(); cC.start(); cL.start(); cx[0].start(priority=1); cF.start(priority=1); cx[1].start(priority=1)

    cb = [pltpu.make_async_copy(b1_hbm, b1_ref, sb.at[0]), pltpu.make_async_copy(b2_hbm, b2_ref, sb.at[1]),
          pltpu.make_async_copy(z_hbm, z_ref, sb.at[2])]

    def bias_setup():
        for c in cb[0:2]:
            c.wait()
        b1f[...] = jnp.broadcast_to(b1_ref[...].astype(F32)[None, :], (8, F))
        b2f[...] = jnp.broadcast_to(b2_ref[...].astype(F32)[None, :], (8, D))
        b1c[...] = jnp.broadcast_to(b1f[:, 1664:F].T[:, 0:1], (64, 128))
    Fk = lambda i: _upk(Fc[:, 128 * i:128 * i + 128])
    Gk = lambda i: _upk(Gc[:, 128 * i:128 * i + 128])

    def wprep(q):
        lo4 = sub < 4
        for tp in range(2):
            outs = []
            for par in range(2):
                tl = 2 * tp + par
                Lm = _upk(L_ref[par])
                o = []
                for k in range(2):
                    Wst[k, par, 0:160, :] = _pk(Wraw[k, q, 0:320, 128 * tl:128 * tl + 128])
                    Wst[k, par, 160:161, :] = pltpu.bitcast(
                        Wraw[k, q, 320:321, 128 * tl:128 * tl + 128].astype(F32), U32) >> 16

                    def tile(cl):
                        ws = []
                        for (rh, rl) in _GROUPS[cl]:
                            w1 = Wst[k, par, pl.ds(rh // 2, 32, stride=5), :]
                            w2 = Wst[k, par, pl.ds(rl // 2, 32, stride=5), :]
                            w1 = (w1 >> 16) if rh % 2 else (w1 & jnp.uint32(0xFFFF))
                            w2 = (w2 & jnp.uint32(0xFFFF0000)) if rl % 2 else (w2 << 16)
                            ws.append(w1 | w2)
                        return jnp.concatenate(ws, axis=0) if len(ws) > 1 else ws[0]
                    t1 = _dot_nt(Lm, _upk(tile(1)))
                    t2 = _dot_nt(Lm, _upk(tile(2)))
                    w0 = tile(0)
                    w0 = jnp.concatenate([w0, w0] if k == 0 else [w0 ^ jnp.uint32(0x80008000), w0], axis=0)
                    t0 = _dot_nt(Lm, _upk(w0))
                    o += [t1, t2, t0]
                outs.append(o)
                yield
            G8 = 8 * (2 * q + tp)
            dst = [(Wr12, 0), (Wr12, 128), (Wa0, 0), (Wi12, 0), (Wi12, 128), (Wb0, 0)]
            for ti in range(6):
                ref, l0 = dst[ti]
                for gam in range(16):
                    A_ = outs[0][ti][8 * gam:8 * gam + 8]; B_ = outs[1][ti][8 * gam:8 * gam + 8]
                    ref[2 * gam, G8:G8 + 8, l0:l0 + 128] = jnp.where(lo4, A_, B_)
                    ref[2 * gam + 1, G8:G8 + 8, l0:l0 + 128] = jnp.where(lo4, B_, A_)
            yield

    sigp = -sig8
    lane64 = lax.broadcasted_iota(jnp.int32, (64, 128), 1)
    lo64 = lane64 < 64
    lo32 = lax.broadcasted_iota(jnp.int32, (32, 128), 1) < 64
    sigalt = jnp.where(lane64 % 2 == 0, 1.0, -1.0).astype(F32)

    zf = {}

    def gate(val, fake):
        if fake is None:
            return val
        return jnp.where(zf['v'], pltpu.bitcast(fake, val.dtype), val)

    def orall(vs):
        vs = [pltpu.bitcast(v, U32) for v in vs]
        while len(vs) > 1:
            vs = [vs[i] | vs[i + 1] if i + 1 < len(vs) else vs[i] for i in range(0, len(vs), 2)]
        return vs[0]

    def vregs(v):
        return [v[8 * i:8 * i + 8, 128 * n:128 * n + 128] for i in range(v.shape[0] // 8) for n in range(v.shape[1] // 128)]

    def gate0(x, fake):
        if fake is None:
            return x
        top = jnp.concatenate([gate(x[0:8, 0:128], fake), x[0:8, 128:]], axis=1)
        return jnp.concatenate([top, x[8:]], axis=0)

    def jp(v):
        return pltpu.roll(v, 64, 1) * sigp

    def rowsum(x):
        return jnp.sum(x, axis=1, keepdims=True)

    def xin(g, a1):
        return jnp.concatenate([XI[g, AORD[8 * a1 + a2]].astype(F32) for a2 in range(8)], axis=0)

    def stC1(g, slot, first=False, chain=False, kara=False):
        fake = None
        for a1 in range(4):
            r0 = 64 * a1
            x = xin(g, a1) if first else X[g, r0:r0 + 64, :]
            x = gate0(x, fake)
            outs = []
            T = [x[:, 128 * a:128 * (a + 1)] for a in range(5)]
            if first or kara:
                t0, t1r, t1i, t2r, t2i = _fwd5k(T)
                k1 = _dot((t1r - t1i).astype(BF), Fk(1)); m1 = _dot(t1i.astype(BF), Fk(2)); n1 = _dot(t1r.astype(BF), Fk(3))
                k2 = _dot((t2r - t2i).astype(BF), Fk(4)); m2 = _dot(t2i.astype(BF), Fk(5)); n2 = _dot(t2r.astype(BF), Fk(6))
            else:
                t0, t1r, t1i, t2r, t2i = _fwd5k([jnp.where(lo64, T[a], T[(a + 2) % 5]) for a in range(5)])
                oo = []
                for i, (R, I) in enumerate(((t1r, t1i), (t2r, t2i))):
                    w2, rw = jnp.where(lo64, R, I), pltpu.roll(jnp.where(lo64, I, R), 64, 1)
                    oo += [_dot((w2 + rw).astype(BF), Fk(7 + 2 * i)), _dot((w2 - rw).astype(BF), Fk(8 + 2 * i))]
            p = (t1r * t1r + t2r * t2r) + (t1i * t1i + t2i * t2i)
            m5 = rowsum(t0) * (1.0 / 128)
            yield
            t0c = t0 - m5
            U0 = _dot(t0c.astype(BF), Fk(0))
            v = rowsum(2.0 * p + t0c * t0c)
            yield
            rs = jnp.exp2(-0.5 * jnp.log2(v * (1.0 / (5 * D)) + 1e-5))
            U0 = U0 * rs
            if first or kara:
                rss = rs * sigalt
                U1 = jnp.concatenate([(k1 + m1) * rs, (k1 - n1) * rss], axis=1)
                U2 = jnp.concatenate([(k2 + m2) * rs, (k2 - n2) * rss], axis=1)
            else:
                U1, U2 = [jnp.concatenate([jnp.where(lo64, oo[i], oo[i + 1]) * rs,
                                           pltpu.roll(jnp.where(lo64, oo[i + 1], oo[i]), 64, 1) * rs], axis=1) for i in (0, 2)]
            x0 = [(U0[8 * a2:8 * a2 + 8], jp(U0[8 * a2:8 * a2 + 8])) for a2 in range(8)]
            for cl, Uc in ((1, U1), (2, U2)):
                xs = [(Uc[8 * a2:8 * a2 + 8, :128], Uc[8 * a2:8 * a2 + 8, 128:]) for a2 in range(8)]
                Y = _fft(xs, _Cplx, -1)
                for c2 in range(8):
                    w = _tw(_Cplx, Y[c2], a1, c2, -1)
                    Ys[slot, 2 * cl - 1, a1, c2] = w[0]; Ys[slot, 2 * cl, a1, c2] = w[1]
                    outs += [w[0], w[1]]
                yield
            Y = _fft(x0, _Cplx, -1)
            for c2 in range(8):
                w = _tw(_Cplx, Y[c2], a1, c2, -1)[0]
                Ys[slot, 0, a1, c2] = w
                outs.append(w)
            if chain:
                fake = orall(outs)
            yield

    def stC2(g, slot, chain=False):
        r0 = pl.multiple_of(8 * g, 8)
        fake = None
        for c2 in range(8):
            y0 = [Ys[slot, 0, a1, c2] for a1 in range(4)]
            y0[0] = gate(y0[0], fake)
            x0 = [(y, jp(y)) for y in y0]
            outs = []
            for cl in (1, 2, 0):
                if cl:
                    xs = [(Ys[slot, 2 * cl - 1, a1, c2], Ys[slot, 2 * cl, a1, c2]) for a1 in range(4)]
                    xs[0] = (gate(xs[0][0], fake), gate(xs[0][1], fake))
                else:
                    xs = x0
                Xo = _fft(xs, _Cplx, -1)
                for c1 in range(4):
                    w = pltpu.pack_elementwise([Xo[c1][0], Xo[c1][1]], packed_dtype=BF)
                    V[c2 + 8 * c1, cl, pl.ds(r0, 8), :] = w
                    outs.append(w)
            if chain:
                fake = orall(outs)
            yield

    def stA1(g, slot, chain=False):
        r0 = pl.multiple_of(8 * g, 8)
        fake = None
        for c2 in range(8):
            h0 = [H0[c2 + 8 * c1, pl.ds(r0, 8), :] for c1 in range(4)]
            h0[0] = gate(h0[0], fake)
            x0 = [(h, jp(h)) for h in h0]
            outs = []
            for cl in (1, 2):
                l0 = 128 * (cl - 1)
                xs = [(H12[c2 + 8 * c1, pl.ds(r0, 8), l0:l0 + 128], H12[c2 + 8 * c1, pl.ds(64 + r0, 8), l0:l0 + 128])
                      for c1 in range(4)]
                xs[0] = (gate(xs[0][0], fake), gate(xs[0][1], fake))
                Zq = _fft(xs, _Cplx, +1)
                for a1 in range(4):
                    v = _tw(_Cplx, Zq[a1], a1, c2, +1)
                    Zs[slot, 2 * cl - 1, a1, c2] = v[0]; Zs[slot, 2 * cl, a1, c2] = v[1]
                    outs += [v[0], v[1]]
            Zq = _fft(x0, _Cplx, +1)
            for a1 in range(4):
                v = _tw(_Cplx, Zq[a1], a1, c2, +1)[0]
                Zs[slot, 0, a1, c2] = v
                outs.append(v)
            if chain:
                fake = orall(outs)
            yield

    def stA2(g, slot, xslot, first=False, chain=False, kara=False):
        fake = None
        for a1 in range(4):
            r0 = 64 * a1
            z0 = [Zs[slot, 0, a1, c2] for c2 in range(8)]
            z0[0] = gate(z0[0], fake)
            x0 = [(z, jp(z)) for z in z0]
            tl = [None] * 5
            for cl in (1, 2):
                Vo = _fft([(Zs[slot, 2 * cl - 1, a1, c2], Zs[slot, 2 * cl, a1, c2]) for c2 in range(8)], _Cplx, +1)
                for ri in range(2):
                    tl[2 * cl - 1 + ri] = jnp.concatenate([o[ri] for o in Vo], axis=0)
            Vo = _fft(x0, _Cplx, +1)
            tl[0] = jnp.concatenate([o[0] for o in Vo], axis=0)
            qs = []
            for cl in (1, 2):
                if kara:
                    vr = tl[2 * cl - 1]; vi = tl[2 * cl] * sigalt
                    o = 3 * cl + 2
                    qs.append((_dot((vr + vi).astype(BF), Gk(o)), _dot(vi.astype(BF), Gk(o + 1)), _dot(vr.astype(BF), Gk(o + 2))))
                    continue
                vr = _pk(tl[2 * cl - 1].astype(BF)); y = pltpu.roll(_pk(tl[2 * cl].astype(BF)), 64, 1)
                qs.append((_dot(_upk(jnp.where(lo32, vr, y)), Gk(2 * cl - 1)), _dot(_upk(jnp.where(lo32, y, vr)), Gk(2 * cl))))
            q0 = _dot(tl[0].astype(BF), Gk(0))
            yield
            if kara:
                ys = _inv5k([q0, qs[0][0] - qs[0][1], qs[0][0] + qs[0][2], qs[1][0] - qs[1][1], qs[1][0] + qs[1][2]])
            else:
                q = [q0]
                for oa, ob in qs:
                    y, y2 = pltpu.roll(oa + ob, 64, 1), oa - ob
                    q += [jnp.where(lo64, y2, y), jnp.where(lo64, y, y2)]
                zz = _inv5k(q)
                ys = [jnp.where(lo64, zz[a], zz[(a + 3) % 5]) for a in range(5)]
            x1 = (xin(g, a1) if first else X[g, r0:r0 + 64, :]) + jnp.concatenate(ys, axis=1)
            X[g, r0:r0 + 64, :] = x1
            m = rowsum(x1) * (1.0 / D)
            yield
            d = X[g, r0:r0 + 64, :] - m
            v = rowsum(d * d)
            yield
            rs = jnp.exp2(-0.5 * jnp.log2(v * (1.0 / D) + 1e-5))
            xn = (X[g, r0:r0 + 64, :] - m) * rs
            XN[xslot, r0:r0 + 64, :] = xn.astype(BF)
            if chain:
                fake = orall(vregs(rs + jnp.zeros((64, 128), F32)))
            yield

    def stB1(g, slot):
        def tchunk():
            hT = _dot_nt(w1_ref[1664:F, :], XN[slot])
            for hh in range(2):
                gT = _gelu(hT[:, 128 * hh:128 * hh + 128] + b1c[...])
                G[128 * hh:128 * hh + 128, 1664:F] = gT.T.astype(BF)
        tpos = 13
        for j in range(14):
            if j == tpos:
                tchunk()
            else:
                jj = j if j < tpos else j - 1
                n0, n1 = 128 * jj, 128 * jj + 128
                h = _dot_nt(XN[slot], w1_ref[n0:n1, :]) + b1f[0:1, n0:n1]
                G[:, n0:n1] = _gelu(h).astype(BF)
            yield

    def stB1s(g, slot):
        for rh in range(2):
            r0 = 128 * rh
            for j in range(13):
                n0, n1 = 128 * j, 128 * j + 128
                h = _dot_nt(XN[slot, r0:r0 + 128, :], w1_ref[n0:n1, :]) + b1f[0:1, n0:n1]
                G[r0:r0 + 128, n0:n1] = _gelu(h).astype(BF)
                yield
        hT = _dot_nt(w1_ref[1664:F, :], XN[slot])
        for hh in range(2):
            gT = _gelu(hT[:, 128 * hh:128 * hh + 128] + b1c[...])
            G[128 * hh:128 * hh + 128, 1664:F] = gT.T.astype(BF)
        yield

    def out_col(g, n):
        return pltpu.make_async_copy(O.at[g, :, :, pl.ds(128 * n, 128)], o_hbm.at[:, g, :, pl.ds(128 * n, 128)], so.at[8 + n])

    def stB2(g, slot, last=False, tail=False):
        for n, rh in [(n, rh) for n in range(5) for rh in range(2)]:
            r0 = 128 * rh
            o = _dot(G[r0:r0 + 128, :], w2_ref[:, 128 * n:128 * n + 128]) + b2f[0:1, 128 * n:128 * n + 128]
            x2 = X[g, r0:r0 + 128, 128 * n:128 * n + 128] + o
            if last:
                for pp in range(16):
                    O[g, AORD[16 * rh + pp], :, 128 * n:128 * n + 128] = x2[8 * pp:8 * pp + 8].astype(BF)
            else:
                X[g, r0:r0 + 128, 128 * n:128 * n + 128] = x2
            if tail and rh == 1:
                out_col(g, n).start()
            yield

    def interleave(main, fillers):
        live = [[f, q, 0.0] for f, q in fillers]
        for _ in main:
            nxt = []
            for e in live:
                e[2] += e[1]
                alive = True
                while e[2] >= 1.0 - 1e-9:
                    e[2] -= 1.0
                    try:
                        next(e[0])
                    except StopIteration:
                        alive = False
                        break
                if alive:
                    nxt.append(e)
            live = nxt
        for e in live:
            _run(e[0])

    sig64 = jnp.where(lax.broadcasted_iota(jnp.int32, (64, 128), 1) < 64, 1.0, -1.0).astype(F32)

    def s_phase(first):
        GP = 2
        NG = NA // GP
        Zq = {}; Y = {}; Hh = {}
        order = [c2 + 8 * c1 for c2 in range(8) for c1 in range(4)]
        cs = lambda p: order[GP * p:GP * p + GP] if 0 <= p < NG else []
        for i in range(NG + 3):
            for c in cs(i - 3):
                h12, h0 = Hh.pop(c)
                H12[c] = h12; H0[c] = h0
            a = {}; b = {}
            for c in cs(i - 2):
                a[c] = _dot(Mi_ref[c], Y[c][0])
            for c in cs(i):
                v12 = jnp.concatenate([_upk(V[c, 1]), _upk(V[c, 2])], axis=1)
                b[c] = _dot(Mf_ref[c], v12)
            for c in cs(i - 2):
                Hh[c] = (a[c], _dot(Mi_ref[c, 0:64], Y.pop(c)[1]))
            for c in cs(i):
                Zq[c] = (b[c], _dot(Mf_ref[c, 0:64], _upk(V[c, 0])))
            for c in cs(i - 1):
                z12, z0 = Zq.pop(c)
                Zr, Zi = z12[0:64], z12[64:128]
                wr = Wr12[c]; wi = Wi12[c]
                y12 = jnp.concatenate([Zr * wr - Zi * wi, Zr * wi + Zi * wr], axis=0).astype(BF)
                y0 = z0 * Wa0[c] + pltpu.roll(z0, 64, 1) * Wb0[c]
                st = jnp.concatenate([y0, pltpu.roll(y0, 64, 1) * sig64], axis=0).astype(BF)
                Y[c] = (y12, st)

    def gen_m():
        cT.wait(); cC.wait(); cL.wait()
        for t in range(2):
            v = TAB[t]
            TAB[2 + t] = jnp.concatenate(
                [v[8 * i + 4 * h:8 * i + 4 * h + 4] for i in range(16) for h in (1, 0)], axis=0)
        Pm = _upk(L_ref[2])
        for c in range(NA):
            o = 2 * (c % 2)
            m = TAB[o] * CS[0, c:c + 1, :] + TAB[o + 1] * CS[1, c:c + 1, :]
            mb = m.astype(BF)
            Mf_ref[c] = mb
            Mi_ref[c] = _dot_nt(Pm, mb).astype(BF)

    with jax.named_scope('ph1'):
        P1 = dict(priority=1)

        def pair(g):
            interleave(stC1(g, g % 4, True), [(stC1(g + 1, (g + 1) % 4, True), 1.0)])
            _run(stC2(g - 2, (g - 2) % 4)); _run(stC2(g - 1, (g - 1) % 4))
        gen_m()
        cx[0].wait()
        for g in range(2, 8):
            cx[g].start(**P1)
        cF.wait(); cx[1].wait()
        for c in cw:
            c.start(**P1)
        for c in cb:
            c.start(**P1)
        interleave(stC1(0, 0, True), [(stC1(1, 1, True), 1.0)])
        for g in (2, 4):
            cx[g].wait(); cx[g + 1].wait()
            if g == 4:
                cG.start(**P1)
                cw1[0].start(**P1)
            pair(g)
        cx[6].wait(); cx[7].wait()
        cw1[1].start(**P1); cw1[2].start(**P1)
        pair(6)
        cw[0].wait(); cw[1].wait(); cw[2].wait(); cw[3].wait(); cb[2].wait()
        zf['v'] = z_ref[0] == 1
        for c_ in cw2[0:2]:
            c_.start(**P1)
        w01 = (y for gen in (wprep(0), wprep(1)) for y in gen)
        interleave(w01, [(stC2(6, 2, True), 0.7), (stC2(7, 3, True), 0.7)])
        cw[4].wait(); cw[5].wait()
        for c_ in cw2[2:5]:
            c_.start(**P1)
        bias_setup()
        _run(wprep(2))
    with jax.named_scope('s1'):
        cw[6].wait(); cw[7].wait(); cG.wait()
        _run(wprep(3))
        s_phase(True)

    def run_plan(mains, fillers):
        i = 0
        for mg in mains:
            for _ in mg:
                for f, plan in fillers:
                    for _ in range(plan[i] if i < len(plan) else 0):
                        try:
                            next(f)
                        except StopIteration:
                            pass
                i += 1
        for f, plan in fillers:
            _run(f)

    def spread(n, lo, hi, tot=24):
        out = [0] * tot
        for i in range(n):
            out[lo + (i * (hi - lo)) // n] += 1
        return out

    def out_copy(g):
        return pltpu.make_async_copy(O.at[g], o_hbm.at[:, g], so.at[g])

    def mlp_phase(last):
        first = not last
        if first:
            for c in cw1:
                c.wait()

        def body0_early():
            _run(stA1(0, 0))
            gA2 = stA2(0, 0, 0, first, kara=True)
            for _ in range(8):
                next(gA2)
            nq = 27
            e0 = 6
            run_plan([stB1s(0, 0)], [(gA2, spread(8, 0, e0, nq)), (stA1(1, 0, True), spread(8, e0 + 2, nq, nq))])
            if first:
                for c in cw2:
                    c.wait()
            run_plan([stB2(0, 0, last)], [(stA2(1, 0, 1, first, True), spread(16, 0, 10, 10))])
            if last:
                out_copy(0).start()

        def body(g, hasC, hasA, tail=False):
            fl = []
            if hasC:
                fl.append((stC1(g - 1, 0, False, True), spread(20, 0, 14)))
                fl.append((stC2(g - 1, 0, True), spread(8, 14, 24)))
            if hasA:
                fl.append((stA1(g + 1, 0, True), spread(8, 0, 14)))
                fl.append((stA2(g + 1, 0, (g + 1) % 2, first, True), spread(16, 14, 24)))
            run_plan([stB1(g, g % 2), stB2(g, g % 2, last, tail)], fl)
            if last and not tail:
                out_copy(g).start()
        body0_early()
        if last:
            lax.fori_loop(1, 7, lambda g, c: (body(g, False, True), c)[1], 0)
            body(7, False, False, tail=True)
        else:
            lax.fori_loop(1, 7, lambda g, c: (body(g, True, True), c)[1], 0)
            body(7, True, False)
            _run(stC1(7, 0, kara=True))
            _run(stC2(7, 0))

    with jax.named_scope('ph2'):
        mlp_phase(False)
    with jax.named_scope('s2'):
        s_phase(False)
    with jax.named_scope('ph3'):
        mlp_phase(True)
    for g in range(7):
        out_copy(g).wait()
    for n in range(5):
        out_col(7, n).wait()


_K = None


@jax.jit
def pallas_interleave_layers__spectral_gfnet__dense_activation_gelu__prompt_kernel(A_x, A_w_r, A_w_i, B_x, B_w1, B_b1, B_w2, B_b2):
    global _K
    if _K is None:
        _K = _build_consts()
    K = _K
    consts = [K[n] for n in ('Fc', 'Gc', 'TAB', 'CS', 'L')]
    any_spec = pl.BlockSpec(memory_space=pl.ANY)
    out = pl.pallas_call(
        _kernel,
        out_shape=jax.ShapeDtypeStruct((NA, 8, 8, D), BF),
        in_specs=[any_spec] * 13,
        out_specs=any_spec,
        scratch_shapes=[
            pltpu.VMEM((8, NA, 8, D), BF),
            pltpu.VMEM((8, NA, 8, D), BF),
            pltpu.VMEM((2, 4, DF, 512), BF),
            pltpu.VMEM((F, D), BF), pltpu.VMEM((F, D), BF),
            pltpu.VMEM((64, 1408), U32), pltpu.VMEM((64, 1408), U32),
            pltpu.VMEM((NA, 128, 128), BF), pltpu.VMEM((NA, 128, 128), BF),
            pltpu.VMEM((3, 64, 128), U32),
            pltpu.VMEM((8, F), F32), pltpu.VMEM((8, D), F32), pltpu.VMEM((64, 128), F32),
            pltpu.VMEM((8, 256, D), F32),
            pltpu.VMEM((NA, 3, 64, 128), U32),
            pltpu.VMEM((NA, 128, 256), F32), pltpu.VMEM((NA, 64, 128), F32),
            pltpu.VMEM((NA, 64, 256), F32), pltpu.VMEM((NA, 64, 256), F32),
            pltpu.VMEM((NA, 64, 128), F32), pltpu.VMEM((NA, 64, 128), F32),
            pltpu.VMEM((2, 2, 168, 128), U32),
            pltpu.VMEM((2, 256, D), BF),
            pltpu.VMEM((256, F), BF),
            pltpu.VMEM((4, 5, 4, 8, 8, 128), F32),
            pltpu.VMEM((2, 5, 4, 8, 8, 128), F32),
            pltpu.VMEM((F,), BF), pltpu.VMEM((D,), BF), pltpu.SMEM((4,), jnp.int32),
            pltpu.VMEM((4, 128, 128), F32), pltpu.VMEM((2, NA, 128), F32),
            pltpu.SemaphoreType.DMA((8,)), pltpu.SemaphoreType.DMA((8,)),
            pltpu.SemaphoreType.DMA((19,)), pltpu.SemaphoreType.DMA((13,)), pltpu.SemaphoreType.DMA((3,)),
        ],
        compiler_params=pltpu.CompilerParams(vmem_limit_bytes=110 * 1024 * 1024),
    )(A_x.reshape(NA, 8, 8, D), A_w_r.T, A_w_i.T, B_w1.T, B_b1, B_w2, B_b2, *consts, np.array([7, 3, 5, 2], dtype=np.int32))
    return out.reshape(1, S, D)
```

```python
import math
import numpy as np
import jax
import jax.numpy as jnp
from jax import lax
import jax.experimental.pallas as pl
import jax.experimental.pallas.tpu as pltpu

S, D, F, DF = 2048, 640, 1728, 321
NA, NB = 32, 64
BF = jnp.bfloat16
F32 = jnp.float32
U32 = jnp.uint32

S1, S2 = math.sin(2 * math.pi / 5), math.sin(4 * math.pi / 5)
K5 = math.sqrt(5.0) / 4.0
R21 = S2 / S1
AORD = [4 * a2 + a1 for a1 in range(4) for a2 in range(8)]


def _fwd5(z):
    z0, z1, z2, z3, z4 = z
    s14 = z1 + z4; d14 = z1 - z4; s23 = z2 + z3; d23 = z2 - z3
    u = s14 + s23
    t0 = z0 + u
    m = z0 - 0.25 * u
    n = K5 * (s14 - s23)
    return t0, m + n, d14 + R21 * d23, m - n, R21 * d14 - d23


_GROUPS = {1: [(6, 4), (1, 9)], 2: [(2, 8), (7, 3)], 0: [(5, 10)]}


def _inv5k(q):
    q0, q1r, q1i, q2r, q2i = q
    u = q1r + q2r
    y0 = q0 + u
    m = q0 - 0.25 * u
    n = K5 * (q1r - q2r)
    a1 = m + n; a2 = m - n
    b1 = S1 * q1i + S2 * q2i
    b2 = S2 * q1i - S1 * q2i
    return y0, a1 - b1, a2 - b2, a2 + b2, a1 + b1


def _fwd5k(z):
    z0, z1, z2, z3, z4 = z
    s14 = z1 + z4; d14 = z1 - z4; s23 = z2 + z3; d23 = z2 - z3
    u = s14 + s23
    t0 = z0 + u
    m = z0 - 0.25 * u
    n = K5 * (s14 - s23)
    return t0, m + n, S1 * d14 + S2 * d23, m - n, S2 * d14 - S1 * d23


def _lane_plan():
    out = {}
    for cl, prs in _GROUPS.items():
        kd = []
        for (rh, rl) in prs:
            for m in range(32):
                kd += [rh + 10 * m, rl + 10 * m]
        out[cl] = np.array(kd, np.int64)
    return out[0], out[1], out[2]


def _build_consts():
    kd0, kd1, kd2 = _lane_plan()
    n = np.arange(D)
    eye = np.eye(D)

    def cs(kd):
        th = 2 * np.pi * np.outer(n, kd) / D
        return np.cos(th), np.sin(th)
    c0, s0 = cs(kd0); c1, s1 = cs(kd1); c2, s2 = cs(kd2)
    s0[:, kd0 == 320] = 0.0
    tiles = [eye[:, 128 * a:128 * (a + 1)] for a in range(5)]
    Ffull = np.concatenate([c0, -s0, c1, -s1, c2, -s2], axis=1)
    Fm = np.linalg.solve(np.concatenate(_fwd5(tiles), axis=1), Ffull)
    kap = lambda kd: np.where(kd == 320, 1.0, 2.0)
    Gfull = np.concatenate([(c0 * kap(kd0)).T, (-s0 * kap(kd0)).T, (c1 * kap(kd1)).T, (-s1 * kap(kd1)).T,
                            (c2 * kap(kd2)).T, (-s2 * kap(kd2)).T], axis=0) / (D * S)
    b = np.arange(64)
    kr = 16 * (b // 8) + 2 * (b % 8); ki = kr + 1
    pos = np.arange(64)
    psi = 2 * np.pi * np.outer(pos, b) / 64
    A0 = np.zeros((128, 128)); B0 = np.zeros((128, 128))
    A0[np.ix_(pos, kr)] = np.cos(psi); A0[np.ix_(pos, ki)] = np.sin(psi)
    A0[np.ix_(64 + pos, kr)] = -np.sin(psi); A0[np.ix_(64 + pos, ki)] = np.cos(psi)
    B0[np.ix_(pos, kr)] = -np.sin(psi); B0[np.ix_(pos, ki)] = np.cos(psi)
    B0[np.ix_(64 + pos, kr)] = -np.cos(psi); B0[np.ix_(64 + pos, ki)] = -np.sin(psi)
    assert np.array_equal(B0, np.concatenate([A0[64:], -A0[:64]]))
    TAB = A0.astype(np.float32)
    phi = 2 * np.pi * np.outer(np.arange(NA), b) / S
    CS = np.zeros((2, NA, 128))
    CS[0][:, kr] = np.cos(phi); CS[0][:, ki] = np.cos(phi)
    CS[1][:, kr] = np.sin(phi); CS[1][:, ki] = np.sin(phi)
    CS = CS.astype(np.float32)
    Pm = np.zeros((128, 128))
    Pm[b, kr] = 1.0; Pm[64 + b, ki] = 1.0
    L = np.zeros((3, 128, 128))
    L[2] = Pm
    for par in range(2):
        for m in range(128):
            gam, j = m // 8, m % 8
            c = 2 * gam + ((j >= 4) if par == 0 else (j < 4))
            L[par, m, c + 32 * (j % 4)] = 1.0
    bf = lambda x: np.asarray(x, dtype=np.float32).astype(BF)
    sg1 = np.where(np.isin(kd1 % 10, (1, 6)), 1.0, -1.0)
    assert np.array_equal(sg1, np.where(np.isin(kd2 % 10, (2, 7)), 1.0, -1.0)) and np.array_equal(sg1, np.tile([1.0, -1.0], 64))
    sg = sg1
    FK = [Fm[0:128, 0:128]]
    for o in (128, 384):
        P = Fm[o:o + 128, o:o + 128]; Q = Fm[o + 128:o + 256, o:o + 128] / S1
        R = Fm[o:o + 128, o + 128:o + 256]; T = Fm[o + 128:o + 256, o + 128:o + 256] / S1
        assert np.abs(T + sg[None, :] * P).max() < 1e-9 and np.abs(R - sg[None, :] * Q).max() < 1e-9
        FK += [P, P + Q, P - Q]
    lo = (np.arange(128) < 64)[None, :]
    sel = lambda a, b: np.where(lo, a, b)
    rol = lambda a: np.roll(a, 64, axis=1)

    def blocks(M):
        out = []
        for i in range(5):
            for j in range(5):
                blk = M[128 * i:128 * i + 128, 128 * j:128 * j + 128]
                if i == j:
                    out.append(blk)
                else:
                    assert np.abs(blk).max() < 1e-9 * np.abs(M).max(), (i, j, np.abs(blk).max())
        return out
    t0, t1r, t1i, t2r, t2i = _fwd5k([sel(tiles[a], tiles[(a + 2) % 5]) for a in range(5)])
    pre = [t0]
    for R, I in ((t1r, t1i), (t2r, t2i)):
        w2, rw = sel(R, I), rol(sel(I, R))
        pre += [w2 + rw, w2 - rw]
    post = [tiles[0]]
    for i in (1, 3):
        post += [sel(tiles[i], tiles[i + 1]), rol(sel(tiles[i + 1], tiles[i]))]
    F5 = blocks(np.linalg.solve(np.concatenate(pre, axis=1), Ffull) @ np.linalg.inv(np.concatenate(post, axis=1)))
    assert np.abs(F5[0] - FK[0]).max() < 1e-9
    FK = np.concatenate(FK + F5[1:], axis=1)
    pre = [tiles[0]]
    for i in (1, 3):
        y = rol(tiles[i + 1])
        pre += [sel(tiles[i], y), sel(y, tiles[i])]
    q = [tiles[0]]
    for i in (1, 3):
        y, y2 = rol(tiles[i] + tiles[i + 1]), tiles[i] - tiles[i + 1]
        q += [sel(y2, y), sel(y, y2)]
    zz = _inv5k(q)
    post = [sel(zz[a], zz[(a + 3) % 5]) for a in range(5)]
    GK = blocks(np.linalg.solve(np.concatenate(pre, axis=1), Gfull) @ np.linalg.inv(np.concatenate(post, axis=1)))
    Gk = np.linalg.solve(np.concatenate(_inv5k(tiles), axis=1).T, Gfull.T).T
    assert np.abs(Gk[0:128, 0:128] - GK[0]).max() < 1e-12
    for o in (128, 384):
        P = Gk[o:o + 128, o:o + 128]; Q = Gk[o + 128:o + 256, o:o + 128]
        R = Gk[o:o + 128, o + 128:o + 256]; T = Gk[o + 128:o + 256, o + 128:o + 256]
        Qt = sg[:, None] * Q; Tt = sg[:, None] * T
        assert np.abs(Tt - P).max() < 1e-12 and np.abs(Qt + R).max() < 1e-12
        GK += [P, P + R, R - P]
    GK = np.concatenate(GK, axis=1)
    def w32(a):
        u = np.asarray(a).view(np.uint16).astype(np.uint32)
        return np.ascontiguousarray(u[..., 0::2, :] | (u[..., 1::2, :] << 16))
    return dict(Fc=w32(bf(FK)), Gc=w32(bf(GK)), TAB=TAB, CS=CS, L=w32(bf(L)))


class _Cplx:
    @staticmethod
    def add(a, b): return (a[0] + b[0], a[1] + b[1])
    @staticmethod
    def sub(a, b): return (a[0] - b[0], a[1] - b[1])
    @staticmethod
    def addsubi(a, b):
        return (a[0] - b[1], a[1] + b[0]), (a[0] + b[1], a[1] - b[0])
    @staticmethod
    def muli(a, sg):
        return (-a[1], a[0]) if sg > 0 else (a[1], -a[0])
    @staticmethod
    def mul(a, c, s):
        if abs(abs(c) - abs(s)) < 1e-12:
            if s * c > 0:
                return (c * (a[0] - a[1]), c * (a[0] + a[1]))
            return (c * (a[0] + a[1]), c * (a[1] - a[0]))
        return (c * a[0] - s * a[1], c * a[1] + s * a[0])


def _fft(x, A, sign):
    N = len(x)
    if N == 1:
        return [x[0]]
    if N == 2:
        return [A.add(x[0], x[1]), A.sub(x[0], x[1])]
    E = _fft(x[0::2], A, sign); O1 = _fft(x[1::4], A, sign); O3 = _fft(x[3::4], A, sign)
    X = [None] * N
    for k in range(N // 4):
        t1, t3 = O1[k], O3[k]
        if k:
            a1 = sign * 2 * math.pi * k / N; a3 = 3 * a1
            t1 = A.mul(t1, math.cos(a1), math.sin(a1)); t3 = A.mul(t3, math.cos(a3), math.sin(a3))
        s = A.add(t1, t3); d = A.sub(t1, t3)
        X[k] = A.add(E[k], s); X[k + N // 2] = A.sub(E[k], s)
        p, m = A.addsubi(E[k + N // 4], d)
        if sign > 0:
            X[k + N // 4], X[k + 3 * N // 4] = p, m
        else:
            X[k + N // 4], X[k + 3 * N // 4] = m, p
    return X


def _tw(A, v, a1, c2, sign):
    n = (a1 * c2) % 32
    if n == 0:
        return v
    if n == 8:
        return A.muli(v, sign)
    ang = sign * 2 * math.pi * n / 32
    return A.mul(v, math.cos(ang), math.sin(ang))


def _dot(a, b):
    return jnp.dot(a, b, preferred_element_type=F32)


def _dot_nt(a, b):
    return lax.dot_general(a, b, (((1,), (1,)), ((), ())), preferred_element_type=F32)


def _gelu(h):
    inner = h * (0.7978845608028654 + (0.7978845608028654 * 0.044715) * (h * h))
    hh = 0.5 * h
    return hh + hh * jnp.tanh(inner)


def _run(gen):
    for _ in gen:
        pass


def _pk(v):
    return pltpu.bitcast(v, U32)


def _upk(w):
    return pltpu.bitcast(w, BF)


def _kernel(x_hbm, wr_hbm, wi_hbm, w1_hbm, b1_hbm, w2_hbm, b2_hbm,
            Fc_hbm, Gc_hbm, TAB_hbm, CS_hbm, L_hbm, z_hbm,
            o_hbm,
            XI, O, Wraw, w1_ref, w2_ref, Fc, Gc, Mf_ref, Mi_ref, L_ref, b1f, b2f, b1c,
            X, V, H12, H0, Wr12, Wi12, Wa0, Wb0, Wst, XN, G, Ys, Zs, b1_ref, b2_ref, z_ref, TAB, CS,
            sx, sw, sm, so, sb):
    lane = lax.broadcasted_iota(jnp.int32, (8, 128), 1)
    sub = lax.broadcasted_iota(jnp.int32, (8, 128), 0)
    lo8 = lane < 64
    sig8 = jnp.where(lo8, -1.0, 1.0).astype(F32)

    cx = [pltpu.make_async_copy(x_hbm.at[:, g], XI.at[g], sx.at[g]) for g in range(8)]
    cw = [pltpu.make_async_copy((wr_hbm, wi_hbm)[k].at[:, pl.ds(512 * q, 512)], Wraw.at[k, q], sw.at[2 * q + k])
          for q in range(4) for k in range(2)]
    cF = pltpu.make_async_copy(Fc_hbm.at[:, pl.ds(0, 896)], Fc.at[:, pl.ds(0, 896)], sm.at[0])
    cF5 = pltpu.make_async_copy(Fc_hbm.at[:, pl.ds(896, 512)], Fc.at[:, pl.ds(896, 512)], sm.at[5])
    cG = pltpu.make_async_copy(Gc_hbm, Gc, sm.at[1])
    cL = pltpu.make_async_copy(L_hbm.at[2], L_ref.at[2], sm.at[2])
    cL2 = pltpu.make_async_copy(L_hbm.at[pl.ds(0, 2)], L_ref.at[pl.ds(0, 2)], sm.at[6])
    cT = pltpu.make_async_copy(TAB_hbm, TAB.at[0], sm.at[3])
    cC = pltpu.make_async_copy(CS_hbm, CS, sm.at[4])
    cw1 = [pltpu.make_async_copy(w1_hbm.at[pl.ds(a, n)], w1_ref.at[pl.ds(a, n)], sm.at[11 + i])
           for i, (a, n) in enumerate(((0, 640), (640, 512), (1152, 576)))]
    cw2 = [pltpu.make_async_copy(w2_hbm.at[:, pl.ds(128 * n, 128)], w2_ref.at[:, pl.ds(128 * n, 128)], sm.at[14 + n])
           for n in range(5)]
    cT.start(); cC.start(); cL.start(); cx[0].start(priority=1); cF.start(priority=1); cx[1].start(priority=1)

    cb = [pltpu.make_async_copy(b1_hbm, b1_ref, sb.at[0]), pltpu.make_async_copy(b2_hbm, b2_ref, sb.at[1]),
          pltpu.make_async_copy(z_hbm, z_ref, sb.at[2])]

    def bias_setup():
        for c in cb[0:2]:
            c.wait()
        b1f[...] = jnp.broadcast_to(b1_ref[...].astype(F32)[None, :], (8, F))
        b2f[...] = jnp.broadcast_to(b2_ref[...].astype(F32)[None, :], (8, D))
        b1c[...] = jnp.broadcast_to(b1f[:, 1664:F].T[:, 0:1], (64, 128))
    Fk = lambda i: _upk(Fc[:, 128 * i:128 * i + 128])
    Gk = lambda i: _upk(Gc[:, 128 * i:128 * i + 128])

    def wprep(q):
        lo4 = sub < 4
        for tp in range(2):
            outs = []
            for par in range(2):
                tl = 2 * tp + par
                Lm = _upk(L_ref[par])
                o = []
                for k in range(2):
                    Wst[k, par, 0:160, :] = _pk(Wraw[k, q, 0:320, 128 * tl:128 * tl + 128])
                    Wst[k, par, 160:161, :] = pltpu.bitcast(
                        Wraw[k, q, 320:321, 128 * tl:128 * tl + 128].astype(F32), U32) >> 16

                    def tile(cl):
                        ws = []
                        for (rh, rl) in _GROUPS[cl]:
                            w1 = Wst[k, par, pl.ds(rh // 2, 32, stride=5), :]
                            w2 = Wst[k, par, pl.ds(rl // 2, 32, stride=5), :]
                            w1 = (w1 >> 16) if rh % 2 else (w1 & jnp.uint32(0xFFFF))
                            w2 = (w2 & jnp.uint32(0xFFFF0000)) if rl % 2 else (w2 << 16)
                            ws.append(w1 | w2)
                        return jnp.concatenate(ws, axis=0) if len(ws) > 1 else ws[0]
                    t1 = _dot_nt(Lm, _upk(tile(1)))
                    t2 = _dot_nt(Lm, _upk(tile(2)))
                    w0 = tile(0)
                    w0 = jnp.concatenate([w0, w0] if k == 0 else [w0 ^ jnp.uint32(0x80008000), w0], axis=0)
                    t0 = _dot_nt(Lm, _upk(w0))
                    o += [t1, t2, t0]
                outs.append(o)
                yield
            G8 = 8 * (2 * q + tp)
            dst = [(Wr12, 0), (Wr12, 128), (Wa0, 0), (Wi12, 0), (Wi12, 128), (Wb0, 0)]
            for ti in range(6):
                ref, l0 = dst[ti]
                for gam in range(16):
                    A_ = outs[0][ti][8 * gam:8 * gam + 8]; B_ = outs[1][ti][8 * gam:8 * gam + 8]
                    ref[2 * gam, G8:G8 + 8, l0:l0 + 128] = jnp.where(lo4, A_, B_)
                    ref[2 * gam + 1, G8:G8 + 8, l0:l0 + 128] = jnp.where(lo4, B_, A_)
            yield

    sigp = -sig8
    lane64 = lax.broadcasted_iota(jnp.int32, (64, 128), 1)
    lo64 = lane64 < 64
    lo32 = lax.broadcasted_iota(jnp.int32, (32, 128), 1) < 64
    sigalt = jnp.where(lane64 % 2 == 0, 1.0, -1.0).astype(F32)

    zf = {}

    def gate(val, fake):
        if fake is None:
            return val
        return jnp.where(zf['v'], pltpu.bitcast(fake, val.dtype), val)

    def orall(vs):
        vs = [pltpu.bitcast(v, U32) for v in vs]
        while len(vs) > 1:
            vs = [vs[i] | vs[i + 1] if i + 1 < len(vs) else vs[i] for i in range(0, len(vs), 2)]
        return vs[0]

    def vregs(v):
        return [v[8 * i:8 * i + 8, 128 * n:128 * n + 128] for i in range(v.shape[0] // 8) for n in range(v.shape[1] // 128)]

    def gate0(x, fake):
        if fake is None:
            return x
        top = jnp.concatenate([gate(x[0:8, 0:128], fake), x[0:8, 128:]], axis=1)
        return jnp.concatenate([top, x[8:]], axis=0)

    def jp(v):
        return pltpu.roll(v, 64, 1) * sigp

    def rowsum(x):
        return jnp.sum(x, axis=1, keepdims=True)

    def xin(g, a1):
        return jnp.concatenate([XI[g, AORD[8 * a1 + a2]].astype(F32) for a2 in range(8)], axis=0)

    def stC1(g, slot, first=False, chain=False, kara=False):
        fake = None
        for a1 in range(4):
            r0 = 64 * a1
            x = xin(g, a1) if first else X[g, r0:r0 + 64, :]
            x = gate0(x, fake)
            outs = []
            T = [x[:, 128 * a:128 * (a + 1)] for a in range(5)]
            if first or kara:
                t0, t1r, t1i, t2r, t2i = _fwd5k(T)
                k1 = _dot((t1r - t1i).astype(BF), Fk(1)); m1 = _dot(t1i.astype(BF), Fk(2)); n1 = _dot(t1r.astype(BF), Fk(3))
                k2 = _dot((t2r - t2i).astype(BF), Fk(4)); m2 = _dot(t2i.astype(BF), Fk(5)); n2 = _dot(t2r.astype(BF), Fk(6))
            else:
                t0, t1r, t1i, t2r, t2i = _fwd5k([jnp.where(lo64, T[a], T[(a + 2) % 5]) for a in range(5)])
                oo = []
                for i, (R, I) in enumerate(((t1r, t1i), (t2r, t2i))):
                    w2, rw = jnp.where(lo64, R, I), pltpu.roll(jnp.where(lo64, I, R), 64, 1)
                    oo += [_dot((w2 + rw).astype(BF), Fk(7 + 2 * i)), _dot((w2 - rw).astype(BF), Fk(8 + 2 * i))]
            p = (t1r * t1r + t2r * t2r) + (t1i * t1i + t2i * t2i)
            m5 = rowsum(t0) * (1.0 / 128)
            yield
            t0c = t0 - m5
            U0 = _dot(t0c.astype(BF), Fk(0))
            v = rowsum(2.0 * p + t0c * t0c)
            yield
            rs = jnp.exp2(-0.5 * jnp.log2(v * (1.0 / (5 * D)) + 1e-5))
            U0 = U0 * rs
            if first or kara:
                rss = rs * sigalt
                U1 = jnp.concatenate([(k1 + m1) * rs, (k1 - n1) * rss], axis=1)
                U2 = jnp.concatenate([(k2 + m2) * rs, (k2 - n2) * rss], axis=1)
            else:
                U1, U2 = [jnp.concatenate([jnp.where(lo64, oo[i], oo[i + 1]) * rs,
                                           pltpu.roll(jnp.where(lo64, oo[i + 1], oo[i]), 64, 1) * rs], axis=1) for i in (0, 2)]
            x0 = [(U0[8 * a2:8 * a2 + 8], jp(U0[8 * a2:8 * a2 + 8])) for a2 in range(8)]
            for cl, Uc in ((1, U1), (2, U2)):
                xs = [(Uc[8 * a2:8 * a2 + 8, :128], Uc[8 * a2:8 * a2 + 8, 128:]) for a2 in range(8)]
                Y = _fft(xs, _Cplx, -1)
                for c2 in range(8):
                    w = _tw(_Cplx, Y[c2], a1, c2, -1)
                    Ys[slot, 2 * cl - 1, a1, c2] = w[0]; Ys[slot, 2 * cl, a1, c2] = w[1]
                    outs += [w[0], w[1]]
                yield
            Y = _fft(x0, _Cplx, -1)
            for c2 in range(8):
                w = _tw(_Cplx, Y[c2], a1, c2, -1)[0]
                Ys[slot, 0, a1, c2] = w
                outs.append(w)
            if chain:
                fake = orall(outs)
            yield

    def stC2(g, slot, chain=False):
        r0 = pl.multiple_of(8 * g, 8)
        fake = None
        for c2 in range(8):
            y0 = [Ys[slot, 0, a1, c2] for a1 in range(4)]
            y0[0] = gate(y0[0], fake)
            x0 = [(y, jp(y)) for y in y0]
            outs = []
            for cl in (1, 2, 0):
                if cl:
                    xs = [(Ys[slot, 2 * cl - 1, a1, c2], Ys[slot, 2 * cl, a1, c2]) for a1 in range(4)]
                    xs[0] = (gate(xs[0][0], fake), gate(xs[0][1], fake))
                else:
                    xs = x0
                Xo = _fft(xs, _Cplx, -1)
                for c1 in range(4):
                    w = pltpu.pack_elementwise([Xo[c1][0], Xo[c1][1]], packed_dtype=BF)
                    V[c2 + 8 * c1, cl, pl.ds(r0, 8), :] = w
                    outs.append(w)
            if chain:
                fake = orall(outs)
            yield

    def stA1(g, slot, chain=False):
        r0 = pl.multiple_of(8 * g, 8)
        fake = None
        for c2 in range(8):
            h0 = [H0[c2 + 8 * c1, pl.ds(r0, 8), :] for c1 in range(4)]
            h0[0] = gate(h0[0], fake)
            x0 = [(h, jp(h)) for h in h0]
            outs = []
            for cl in (1, 2):
                l0 = 128 * (cl - 1)
                xs = [(H12[c2 + 8 * c1, pl.ds(r0, 8), l0:l0 + 128], H12[c2 + 8 * c1, pl.ds(64 + r0, 8), l0:l0 + 128])
                      for c1 in range(4)]
                xs[0] = (gate(xs[0][0], fake), gate(xs[0][1], fake))
                Zq = _fft(xs, _Cplx, +1)
                for a1 in range(4):
                    v = _tw(_Cplx, Zq[a1], a1, c2, +1)
                    Zs[slot, 2 * cl - 1, a1, c2] = v[0]; Zs[slot, 2 * cl, a1, c2] = v[1]
                    outs += [v[0], v[1]]
            Zq = _fft(x0, _Cplx, +1)
            for a1 in range(4):
                v = _tw(_Cplx, Zq[a1], a1, c2, +1)[0]
                Zs[slot, 0, a1, c2] = v
                outs.append(v)
            if chain:
                fake = orall(outs)
            yield

    def stA2(g, slot, xslot, first=False, chain=False, kara=False):
        fake = None
        for a1 in range(4):
            r0 = 64 * a1
            z0 = [Zs[slot, 0, a1, c2] for c2 in range(8)]
            z0[0] = gate(z0[0], fake)
            x0 = [(z, jp(z)) for z in z0]
            tl = [None] * 5
            for cl in (1, 2):
                Vo = _fft([(Zs[slot, 2 * cl - 1, a1, c2], Zs[slot, 2 * cl, a1, c2]) for c2 in range(8)], _Cplx, +1)
                for ri in range(2):
                    tl[2 * cl - 1 + ri] = jnp.concatenate([o[ri] for o in Vo], axis=0)
            Vo = _fft(x0, _Cplx, +1)
            tl[0] = jnp.concatenate([o[0] for o in Vo], axis=0)
            qs = []
            for cl in (1, 2):
                if kara:
                    vr = tl[2 * cl - 1]; vi = tl[2 * cl] * sigalt
                    o = 3 * cl + 2
                    qs.append((_dot((vr + vi).astype(BF), Gk(o)), _dot(vi.astype(BF), Gk(o + 1)), _dot(vr.astype(BF), Gk(o + 2))))
                    continue
                vr = _pk(tl[2 * cl - 1].astype(BF)); y = pltpu.roll(_pk(tl[2 * cl].astype(BF)), 64, 1)
                qs.append((_dot(_upk(jnp.where(lo32, vr, y)), Gk(2 * cl - 1)), _dot(_upk(jnp.where(lo32, y, vr)), Gk(2 * cl))))
            q0 = _dot(tl[0].astype(BF), Gk(0))
            yield
            if kara:
                ys = _inv5k([q0, qs[0][0] - qs[0][1], qs[0][0] + qs[0][2], qs[1][0] - qs[1][1], qs[1][0] + qs[1][2]])
            else:
                q = [q0]
                for oa, ob in qs:
                    y, y2 = pltpu.roll(oa + ob, 64, 1), oa - ob
                    q += [jnp.where(lo64, y2, y), jnp.where(lo64, y, y2)]
                zz = _inv5k(q)
                ys = [jnp.where(lo64, zz[a], zz[(a + 3) % 5]) for a in range(5)]
            x1 = (xin(g, a1) if first else X[g, r0:r0 + 64, :]) + jnp.concatenate(ys, axis=1)
            X[g, r0:r0 + 64, :] = x1
            m = rowsum(x1) * (1.0 / D)
            yield
            d = X[g, r0:r0 + 64, :] - m
            v = rowsum(d * d)
            yield
            rs = jnp.exp2(-0.5 * jnp.log2(v * (1.0 / D) + 1e-5))
            xn = (X[g, r0:r0 + 64, :] - m) * rs
            XN[xslot, r0:r0 + 64, :] = xn.astype(BF)
            if chain:
                fake = orall(vregs(rs + jnp.zeros((64, 128), F32)))
            yield

    def stB1(g, slot):
        def tchunk():
            hT = _dot_nt(w1_ref[1664:F, :], XN[slot])
            for hh in range(2):
                gT = _gelu(hT[:, 128 * hh:128 * hh + 128] + b1c[...])
                G[128 * hh:128 * hh + 128, 1664:F] = gT.T.astype(BF)
        tpos = 13
        for j in range(14):
            if j == tpos:
                tchunk()
            else:
                jj = j if j < tpos else j - 1
                n0, n1 = 128 * jj, 128 * jj + 128
                h = _dot_nt(XN[slot], w1_ref[n0:n1, :]) + b1f[0:1, n0:n1]
                G[:, n0:n1] = _gelu(h).astype(BF)
            yield

    def stB1s(g, slot):
        for rh in range(2):
            r0 = 128 * rh
            for j in range(13):
                n0, n1 = 128 * j, 128 * j + 128
                h = _dot_nt(XN[slot, r0:r0 + 128, :], w1_ref[n0:n1, :]) + b1f[0:1, n0:n1]
                G[r0:r0 + 128, n0:n1] = _gelu(h).astype(BF)
                yield
        hT = _dot_nt(w1_ref[1664:F, :], XN[slot])
        for hh in range(2):
            gT = _gelu(hT[:, 128 * hh:128 * hh + 128] + b1c[...])
            G[128 * hh:128 * hh + 128, 1664:F] = gT.T.astype(BF)
        yield

    def out_col(g, n):
        return pltpu.make_async_copy(O.at[g, :, :, pl.ds(128 * n, 128)], o_hbm.at[:, g, :, pl.ds(128 * n, 128)], so.at[8 + n])

    def stB2(g, slot, last=False, tail=False):
        for n, rh in [(n, rh) for n in range(5) for rh in range(2)]:
            r0 = 128 * rh
            o = _dot(G[r0:r0 + 128, :], w2_ref[:, 128 * n:128 * n + 128]) + b2f[0:1, 128 * n:128 * n + 128]
            x2 = X[g, r0:r0 + 128, 128 * n:128 * n + 128] + o
            if last:
                for pp in range(16):
                    O[g, AORD[16 * rh + pp], :, 128 * n:128 * n + 128] = x2[8 * pp:8 * pp + 8].astype(BF)
            else:
                X[g, r0:r0 + 128, 128 * n:128 * n + 128] = x2
            if tail and rh == 1:
                out_col(g, n).start()
            yield

    def interleave(main, fillers):
        live = [[f, q, 0.0] for f, q in fillers]
        for _ in main:
            nxt = []
            for e in live:
                e[2] += e[1]
                alive = True
                while e[2] >= 1.0 - 1e-9:
                    e[2] -= 1.0
                    try:
                        next(e[0])
                    except StopIteration:
                        alive = False
                        break
                if alive:
                    nxt.append(e)
            live = nxt
        for e in live:
            _run(e[0])

    sig64 = jnp.where(lax.broadcasted_iota(jnp.int32, (64, 128), 1) < 64, 1.0, -1.0).astype(F32)

    def s_phase(first):
        GP = 2
        NG = NA // GP
        Zq = {}; Y = {}; Hh = {}
        order = [c2 + 8 * c1 for c2 in range(8) for c1 in range(4)]
        cs = lambda p: order[GP * p:GP * p + GP] if 0 <= p < NG else []
        for i in range(NG + 3):
            for c in cs(i - 3):
                h12, h0 = Hh.pop(c)
                H12[c] = h12; H0[c] = h0
            a = {}; b = {}
            for c in cs(i - 2):
                a[c] = _dot(Mi_ref[c], Y[c][0])
            for c in cs(i):
                v12 = jnp.concatenate([_upk(V[c, 1]), _upk(V[c, 2])], axis=1)
                b[c] = _dot(Mf_ref[c], v12)
            for c in cs(i - 2):
                Hh[c] = (a[c], _dot(Mi_ref[c, 0:64], Y.pop(c)[1]))
            for c in cs(i):
                Zq[c] = (b[c], _dot(Mf_ref[c, 0:64], _upk(V[c, 0])))
            for c in cs(i - 1):
                z12, z0 = Zq.pop(c)
                Zr, Zi = z12[0:64], z12[64:128]
                wr = Wr12[c]; wi = Wi12[c]
                y12 = jnp.concatenate([Zr * wr - Zi * wi, Zr * wi + Zi * wr], axis=0).astype(BF)
                y0 = z0 * Wa0[c] + pltpu.roll(z0, 64, 1) * Wb0[c]
                st = jnp.concatenate([y0, pltpu.roll(y0, 64, 1) * sig64], axis=0).astype(BF)
                Y[c] = (y12, st)

    def gen_m():
        cT.wait(); cC.wait(); cL.wait()
        TAB[1] = jnp.concatenate([TAB[0, 64:128], -TAB[0, 0:64]], axis=0)
        for t in range(2):
            v = TAB[t]
            TAB[2 + t] = jnp.concatenate(
                [v[8 * i + 4 * h:8 * i + 4 * h + 4] for i in range(16) for h in (1, 0)], axis=0)
        Pm = _upk(L_ref[2])
        for c in range(NA):
            o = 2 * (c % 2)
            m = TAB[o] * CS[0, c:c + 1, :] + TAB[o + 1] * CS[1, c:c + 1, :]
            mb = m.astype(BF)
            Mf_ref[c] = mb
            Mi_ref[c] = _dot_nt(Pm, mb).astype(BF)

    with jax.named_scope('ph1'):
        P1 = dict(priority=1)

        def pair(g):
            interleave(stC1(g, g % 4, True), [(stC1(g + 1, (g + 1) % 4, True), 1.0)])
            _run(stC2(g - 2, (g - 2) % 4)); _run(stC2(g - 1, (g - 1) % 4))
        gen_m()
        cL2.start(**P1)
        cx[0].wait()
        for g in range(2, 8):
            cx[g].start(**P1)
        cF.wait(); cx[1].wait()
        for c in cw:
            c.start(**P1)
        for c in cb:
            c.start(**P1)
        interleave(stC1(0, 0, True), [(stC1(1, 1, True), 1.0)])
        for g in (2, 4):
            cx[g].wait(); cx[g + 1].wait()
            if g == 4:
                cG.start(**P1)
                cF5.start(**P1)
                cw1[0].start(**P1)
            pair(g)
        cx[6].wait(); cx[7].wait()
        cw1[1].start(**P1); cw1[2].start(**P1)
        pair(6)
        cw[0].wait(); cw[1].wait(); cw[2].wait(); cw[3].wait(); cb[2].wait(); cL2.wait()
        zf['v'] = z_ref[0] == 1
        for c_ in cw2[0:2]:
            c_.start(**P1)
        w01 = (y for gen in (wprep(0), wprep(1)) for y in gen)
        interleave(w01, [(stC2(6, 2, True), 0.7), (stC2(7, 3, True), 0.7)])
        cw[4].wait(); cw[5].wait()
        for c_ in cw2[2:5]:
            c_.start(**P1)
        bias_setup()
        _run(wprep(2))
    with jax.named_scope('s1'):
        cw[6].wait(); cw[7].wait()
        _run(wprep(3))
        s_phase(True)

    def run_plan(mains, fillers):
        i = 0
        for mg in mains:
            for _ in mg:
                for f, plan in fillers:
                    for _ in range(plan[i] if i < len(plan) else 0):
                        try:
                            next(f)
                        except StopIteration:
                            pass
                i += 1
        for f, plan in fillers:
            _run(f)

    def spread(n, lo, hi, tot=24):
        out = [0] * tot
        for i in range(n):
            out[lo + (i * (hi - lo)) // n] += 1
        return out

    def out_copy(g):
        return pltpu.make_async_copy(O.at[g], o_hbm.at[:, g], so.at[g])

    def mlp_phase(last):
        first = not last
        if first:
            for c in cw1 + [cG, cF5]:
                c.wait()

        def body0_early():
            _run(stA1(0, 0))
            gA2 = stA2(0, 0, 0, first, kara=True)
            for _ in range(8):
                next(gA2)
            nq = 27
            e0 = 6
            run_plan([stB1s(0, 0)], [(gA2, spread(8, 0, e0, nq)), (stA1(1, 0, True), spread(8, e0 + 2, nq, nq))])
            if first:
                for c in cw2:
                    c.wait()
            run_plan([stB2(0, 0, last)], [(stA2(1, 0, 1, first, True), spread(16, 0, 10, 10))])
            if last:
                out_copy(0).start()

        def body(g, hasC, hasA, tail=False):
            fl = []
            if hasC:
                fl.append((stC1(g - 1, 0, False, True), spread(20, 0, 14)))
                fl.append((stC2(g - 1, 0, True), spread(8, 14, 24)))
            if hasA:
                fl.append((stA1(g + 1, 0, True), spread(8, 0, 14)))
                fl.append((stA2(g + 1, 0, (g + 1) % 2, first, True), spread(16, 14, 24)))
            run_plan([stB1(g, g % 2), stB2(g, g % 2, last, tail)], fl)
            if last and not tail:
                out_copy(g).start()
        body0_early()
        if last:
            lax.fori_loop(1, 7, lambda g, c: (body(g, False, True), c)[1], 0)
            body(7, False, False, tail=True)
        else:
            lax.fori_loop(1, 7, lambda g, c: (body(g, True, True), c)[1], 0)
            body(7, True, False)
            _run(stC1(7, 0, kara=True))
            _run(stC2(7, 0))

    with jax.named_scope('ph2'):
        mlp_phase(False)
    with jax.named_scope('s2'):
        s_phase(False)
    with jax.named_scope('ph3'):
        mlp_phase(True)
    for g in range(7):
        out_copy(g).wait()
    for n in range(5):
        out_col(7, n).wait()


_K = None


@jax.jit
def pallas_interleave_layers__spectral_gfnet__dense_activation_gelu__prompt_kernel(A_x, A_w_r, A_w_i, B_x, B_w1, B_b1, B_w2, B_b2):
    global _K
    if _K is None:
        _K = _build_consts()
    K = _K
    consts = [K[n] for n in ('Fc', 'Gc', 'TAB', 'CS', 'L')]
    any_spec = pl.BlockSpec(memory_space=pl.ANY)
    out = pl.pallas_call(
        _kernel,
        out_shape=jax.ShapeDtypeStruct((NA, 8, 8, D), BF),
        in_specs=[any_spec] * 13,
        out_specs=any_spec,
        scratch_shapes=[
            pltpu.VMEM((8, NA, 8, D), BF),
            pltpu.VMEM((8, NA, 8, D), BF),
            pltpu.VMEM((2, 4, DF, 512), BF),
            pltpu.VMEM((F, D), BF), pltpu.VMEM((F, D), BF),
            pltpu.VMEM((64, 1408), U32), pltpu.VMEM((64, 1408), U32),
            pltpu.VMEM((NA, 128, 128), BF), pltpu.VMEM((NA, 128, 128), BF),
            pltpu.VMEM((3, 64, 128), U32),
            pltpu.VMEM((8, F), F32), pltpu.VMEM((8, D), F32), pltpu.VMEM((64, 128), F32),
            pltpu.VMEM((8, 256, D), F32),
            pltpu.VMEM((NA, 3, 64, 128), U32),
            pltpu.VMEM((NA, 128, 256), F32), pltpu.VMEM((NA, 64, 128), F32),
            pltpu.VMEM((NA, 64, 256), F32), pltpu.VMEM((NA, 64, 256), F32),
            pltpu.VMEM((NA, 64, 128), F32), pltpu.VMEM((NA, 64, 128), F32),
            pltpu.VMEM((2, 2, 168, 128), U32),
            pltpu.VMEM((2, 256, D), BF),
            pltpu.VMEM((256, F), BF),
            pltpu.VMEM((4, 5, 4, 8, 8, 128), F32),
            pltpu.VMEM((2, 5, 4, 8, 8, 128), F32),
            pltpu.VMEM((F,), BF), pltpu.VMEM((D,), BF), pltpu.SMEM((4,), jnp.int32),
            pltpu.VMEM((4, 128, 128), F32), pltpu.VMEM((2, NA, 128), F32),
            pltpu.SemaphoreType.DMA((8,)), pltpu.SemaphoreType.DMA((8,)),
            pltpu.SemaphoreType.DMA((19,)), pltpu.SemaphoreType.DMA((13,)), pltpu.SemaphoreType.DMA((3,)),
        ],
        compiler_params=pltpu.CompilerParams(vmem_limit_bytes=110 * 1024 * 1024),
    )(A_x.reshape(NA, 8, 8, D), A_w_r.T, A_w_i.T, B_w1.T, B_b1, B_w2, B_b2, *consts, np.array([7, 3, 5, 2], dtype=np.int32))
    return out.reshape(1, S, D)
```
